```python
import os as _os
_os.environ.setdefault('JAX_PLATFORMS', 'cpu')
import jax
import jax.numpy as jnp

def _softmax(x, axis=-1):
    return jax.nn.softmax(x, axis=axis)

def _gelu(x):
    return jax.nn.gelu(x, approximate=True)

def _silu(x):
    return jax.nn.silu(x)

def _sigmoid(x):
    return jax.nn.sigmoid(x)

def _layernorm(x, axis=-1, eps=1e-05):
    m = jnp.mean(x, axis=axis, keepdims=True)
    v = jnp.var(x, axis=axis, keepdims=True)
    return (x - m) / jnp.sqrt(v + eps)

def _scatter_add(tgt, idx, src, axis=0):
    return tgt.at[idx].add(src)

def _segment_sum(src, seg, n):
    return jax.ops.segment_sum(src, seg, n)

class _Rng:

    def __init__(self, key):
        self._k = key

    def _next(self):
        self._k, sub = jax.random.split(self._k)
        return sub

    def normal(self, shape):
        return jax.random.normal(self._next(), shape, dtype=jnp.bfloat16)

    def randint(self, lo, hi, shape):
        return jax.random.randint(self._next(), shape, lo, hi, dtype=jnp.int32)

    def uniform(self, shape, lo=0.0, hi=1.0):
        return jax.random.uniform(self._next(), shape, jnp.bfloat16, lo, hi)

    def permutation(self, n):
        return jax.random.permutation(self._next(), n)
kernel_name = 'adaLN_cond__grouped_kv_mqa__swiglu_ffn__prompt'

def setup_inputs():
    _rng = _Rng(jax.random.key(int.from_bytes(__import__("os").urandom(4), "little")))
    _w = lambda a: (lambda t: t.astype(jnp.bfloat16) if jnp.issubdtype(t.dtype, jnp.floating) else t)(jnp.asarray(a))

    def _A_setup():
        B, S, D, H = (1, 2048, 576, 32)
        Dh = D // H
        return {'x': _w((lambda *s: _rng.normal(s) * 0.05)(B, S, D)), 'wq': _w((lambda *s: _rng.normal(s) * 0.05)(D, H * Dh)), 'wk': _w((lambda *s: _rng.normal(s) * 0.05)(D, Dh)), 'wv': _w((lambda *s: _rng.normal(s) * 0.05)(D, Dh)), 'wo': _w((lambda *s: _rng.normal(s) * 0.05)(H * Dh, D))}
    _A_in = _A_setup()

    def _B_setup():
        B, S, D, F = (1, 2048, 576, 4608)
        return {'x': _w((lambda *s: _rng.normal(s) * 0.05)(B, S, D)), 'w_gate': _w((lambda *s: _rng.normal(s) * 0.05)(D, F)), 'w_up': _w((lambda *s: _rng.normal(s) * 0.05)(D, F)), 'w_down': _w((lambda *s: _rng.normal(s) * 0.05)(F, D))}
    _B_in = _B_setup()
    return {'A_x': _A_in['x'], 'A_wq': _A_in['wq'], 'A_wk': _A_in['wk'], 'A_wv': _A_in['wv'], 'A_wo': _A_in['wo'], 'B_x': _B_in['x'], 'B_w_gate': _B_in['w_gate'], 'B_w_up': _B_in['w_up'], 'B_w_down': _B_in['w_down'], 'c': _w((lambda *s: _rng.normal(s) * 0.05)(1, 576) * 8.0), 'w_mod': _w((lambda *s: _rng.normal(s) * 0.05)(576, 6 * 576) * 576 ** (-0.5) * 8.0)}

def reference(A_x, A_wq, A_wk, A_wv, A_wo, B_x, B_w_gate, B_w_up, B_w_down, c, w_mod):

    def _A_ref(x, wq, wk, wv, wo):
        B, S, D = x.shape
        H = 32
        Dh = D // H
        q = (lambda x, *d: x.transpose(*d))((x @ wq).reshape(B, S, H, Dh), 0, 2, 1, 3)
        k = x @ wk
        v = x @ wv
        scores = jnp.einsum('bhqd,bkd->bhqk', q, k) * Dh ** (-0.5)
        p = _softmax(scores, axis=-1)
        o = jnp.einsum('bhqk,bkd->bhqd', p, v)
        return (lambda x, *d: x.transpose(*d))(o, 0, 2, 1, 3).reshape(B, S, H * Dh) @ wo

    def _B_ref(x, w_gate, w_up, w_down):
        g = _silu(x @ w_gate)
        u = x @ w_up
        return g * u @ w_down
    x = A_x
    mod = (_silu(c) @ w_mod).reshape(c.shape[0], 6, 1, -1)
    sa, ca, ga, sb, cb, gb = (mod[:, 0].copy(), mod[:, 1].copy(), mod[:, 2].copy(), mod[:, 3].copy(), mod[:, 4].copy(), mod[:, 5].copy())
    h = _layernorm(x, axis=-1) * (1 + ca) + sa
    x = x + ga * _A_ref(h, A_wq, A_wk, A_wv, A_wo)
    h = _layernorm(x, axis=-1) * (1 + cb) + sb
    x = x + gb * _B_ref(h, B_w_gate, B_w_up, B_w_down)
    return x
```

```python
import math

import jax
import jax.numpy as jnp
import jax.experimental.pallas as pl
import jax.experimental.pallas.tpu as pltpu

F32 = jnp.float32
BF16 = jnp.bfloat16

S = 2048
D = 576
H = 32
DH = D // H
FF = 4608
EPS = 1e-05

KW = 24
VR = 24
NQKV = D + 2 * KW

TQ = 512
NQB = S // TQ
KC = 128
HPI = 4
NG = H // HPI
FC = 768
NFC = FF // FC
MOD1 = 2 * D

QK_SCALE = (DH ** -0.5) * math.log2(math.e)


def _dot(a, b):
    return jnp.dot(a, b, preferred_element_type=F32)


def _dot_nt(a, b):
    return jax.lax.dot_general(a, b, (((1,), (1,)), ((), ())), preferred_element_type=F32)


def _ln_t(x):
    m = jnp.mean(x, axis=0, keepdims=True)
    xc = x - m
    v = jnp.mean(xc * xc, axis=0, keepdims=True)
    return xc * jax.lax.rsqrt(v + EPS)


def _silu(g):
    return g * (1.0 / (1.0 + jnp.exp(-g)))


def _lanes(col, n):
    return jnp.concatenate([col] * (n // 128), axis=1)


def _kernel(
    xt_hbm, wq_hbm, wkt_hbm, wvt_hbm, wo_hbm, wg_hbm, wu_hbm, wdt_hbm, c_hbm, wmod_hbm,
    out_hbm,
    xt_ref, wq_ref, wkt_ref, wvt_ref, wo_ref, wg_ref, wu_ref, wdt_ref, c_ref, wmod_ref,
    in_sems, x_sems, out_sems,
    mod_ref, wqkv_ref, wot_ref, ks_ref, vt_ref, qt_ref, s_ref, m_ref, ot_ref,
    x1_ref, h2_ref, acc_ref, stage_ref,
):
    def copy(src, dst, sem):
        return pltpu.make_async_copy(src, dst, sem)

    cp_c = copy(c_hbm, c_ref, in_sems.at[0])
    cp_m1 = copy(wmod_hbm.at[:, pl.ds(0, MOD1)], wmod_ref.at[:, pl.ds(0, MOD1)], in_sems.at[1])
    cp_q = copy(wq_hbm, wq_ref, in_sems.at[2])
    cp_k = copy(wkt_hbm, wkt_ref, in_sems.at[3])
    cp_v = copy(wvt_hbm, wvt_ref, in_sems.at[4])
    cp_x = [copy(xt_hbm.at[0, :, pl.ds(i * TQ, TQ)], xt_ref.at[i], x_sems.at[i]) for i in range(NQB)]
    cp_o = copy(wo_hbm, wo_ref, in_sems.at[5])
    cp_m2 = copy(wmod_hbm.at[:, pl.ds(MOD1, 6 * D - MOD1)], wmod_ref.at[:, pl.ds(MOD1, 6 * D - MOD1)],
                 in_sems.at[6])
    cp_g = copy(wg_hbm, wg_ref, in_sems.at[7])
    cp_u = copy(wu_hbm, wu_ref, in_sems.at[8])
    cp_d = copy(wdt_hbm, wdt_ref, in_sems.at[9])

    cp_c.start()
    cp_q.start()
    cp_k.start()
    cp_v.start()
    cp_m1.start()
    for cp in cp_x:
        cp.start()

    cp_q.wait()
    cp_k.wait()
    cp_v.wait()
    wqkv_ref[0:D, :] = wq_ref[...].astype(F32).T.astype(BF16)
    zpad = jnp.zeros((KW - DH, D), F32)
    kv_t = jnp.concatenate(
        [wkt_ref[...].astype(F32), zpad, wvt_ref[...].astype(F32), zpad], axis=0)
    wqkv_ref[D:NQKV, :] = kv_t.astype(BF16)

    cp_c.wait()
    sc = jnp.broadcast_to(_silu(c_ref[...].astype(F32)), (8, D))

    def mod_cols(lo, hi):
        mod = _dot(sc, wmod_ref[:, lo:hi])
        mod_ref[lo:hi, :] = jnp.broadcast_to(mod[0:1, :], (128, hi - lo)).T

    cp_m1.wait()
    mod_cols(0, MOD1)

    for i in range(NQB):
        cp_x[i].wait()
        if i == NQB - 1:
            cp_o.start()
            cp_m2.start()
            cp_g.start()
            cp_u.start()
            cp_d.start()
        sa = _lanes(mod_ref[0:D, :], TQ)
        ca1 = 1.0 + _lanes(mod_ref[D:2 * D, :], TQ)
        h = (_ln_t(xt_ref[i].astype(F32)) * ca1 + sa).astype(BF16)
        qkv = _dot(wqkv_ref[...], h)
        qt_ref[i] = qkv[0:D, :]
        row = jax.lax.broadcasted_iota(jnp.int32, (VR, TQ), 0)
        vt_ref[:, i * TQ:(i + 1) * TQ] = jnp.where(row == DH, 1.0, qkv[D + KW:NQKV, :])
        kt = jnp.concatenate(
            [qkv[D:D + KW, :] * QK_SCALE, jnp.zeros((128 - KW, TQ), F32)], axis=0)
        k = kt.T
        for r in range(HPI):
            kr = k if r == 0 else pltpu.roll(k, 2 * r, 1)
            ks_ref[r, i * TQ:(i + 1) * TQ, :] = kr[:, 0:KW].astype(BF16)

    def q_window(g, r):
        base = (g % NG) * (HPI * DH) + 16 * r
        return qt_ref[g // NG, pl.ds(pl.multiple_of(base, 8), KW), :]

    def step(q, r, slot_q, slot_p):
        mp = m_ref[slot_p]
        m = None
        acc = None
        for cidx in range(S // KC):
            sl = pl.ds(cidx * KC, KC)
            if q is not None:
                s = _dot(ks_ref[r, sl, :], q)
                s_ref[slot_q, sl, :] = s
                mc = jnp.max(s.reshape(KC // 8, 8, TQ), axis=0)
                m = mc if m is None else jnp.maximum(m, mc)
            p = jnp.exp2(s_ref[slot_p, sl, :] - mp).astype(BF16)
            o = _dot(vt_ref[:, sl], p)
            acc = o if acc is None else acc + o
        if q is not None:
            m_ref[slot_q] = jnp.max(m, axis=0, keepdims=True)
        return acc[0:DH, :] * (1.0 / acc[DH:DH + 1, :])

    s0 = _dot(ks_ref[0], q_window(0, 0))
    s_ref[0] = s0
    m_ref[0] = jnp.max(s0, axis=0, keepdims=True)

    def group(g, last):
        outs = []
        for u in range(HPI):
            r = (u + 1) % HPI
            if u < HPI - 1:
                q = q_window(g, r)
            else:
                q = None if last else q_window(g + 1, r)
            outs.append(step(q, r, (u + 1) % 2, u % 2))
        off = pl.multiple_of((g % NG) * (HPI * DH), 8)
        ot_ref[g // NG, pl.ds(off, HPI * DH), :] = jnp.concatenate(outs, axis=0)

    def phase_b(g, carry):
        group(g, False)
        return carry

    jax.lax.fori_loop(0, NQB * NG - 1, phase_b, 0)

    cp_o.wait()
    cp_m2.wait()
    group(NQB * NG - 1, True)

    wot_ref[...] = wo_ref[...].astype(F32).T.astype(BF16)
    mod_cols(MOD1, 6 * D)

    for i in range(NQB):
        ga = _lanes(mod_ref[2 * D:3 * D, :], TQ)
        sb = _lanes(mod_ref[3 * D:4 * D, :], TQ)
        cb1 = 1.0 + _lanes(mod_ref[4 * D:5 * D, :], TQ)
        attn = _dot(wot_ref[...], ot_ref[i])
        x1 = xt_ref[i].astype(F32) + ga * attn
        x1_ref[i] = x1
        h2_ref[i] = (_ln_t(x1) * cb1 + sb).T.astype(BF16)
        acc_ref[i] = jnp.zeros((D, TQ), F32)

    cp_g.wait()
    cp_u.wait()
    cp_d.wait()

    def out_copy(mb):
        return copy(stage_ref.at[mb],
                    out_hbm.at[0, :, pl.ds(pl.multiple_of(mb * TQ, TQ), TQ)],
                    out_sems.at[mb])

    def phase_d(i, carry):
        mb = i // NFC
        fc = i % NFC
        cols = pl.ds(pl.multiple_of(fc * FC, FC), FC)
        h = h2_ref[mb]
        g = _dot(h, wg_ref[:, cols])
        u = _dot(h, wu_ref[:, cols])
        a = (_silu(g) * u).astype(BF16)
        acc_ref[mb] += _dot_nt(wdt_ref[:, cols], a)

        @pl.when(fc == NFC - 1)
        def _():
            gb = _lanes(mod_ref[5 * D:6 * D, :], TQ)
            stage_ref[mb] = (x1_ref[mb] + gb * acc_ref[mb]).astype(BF16)
            out_copy(mb).start()

        return carry

    jax.lax.fori_loop(0, NQB * NFC, phase_d, 0)
    for mb in range(NQB):
        out_copy(mb).wait()


@jax.jit
def pallas_adaLN_cond__grouped_kv_mqa__swiglu_ffn__prompt_kernel(
    A_x: jax.Array,
    A_wq: jax.Array,
    A_wk: jax.Array,
    A_wv: jax.Array,
    A_wo: jax.Array,
    B_x: jax.Array,
    B_w_gate: jax.Array,
    B_w_up: jax.Array,
    B_w_down: jax.Array,
    c: jax.Array,
    w_mod: jax.Array,
):
    del B_x
    hbm = pl.BlockSpec(memory_space=pltpu.HBM)
    out_t = pl.pallas_call(
        _kernel,
        out_shape=jax.ShapeDtypeStruct((1, D, S), A_x.dtype),
        in_specs=[hbm] * 10,
        out_specs=hbm,
        scratch_shapes=[
            pltpu.VMEM((NQB, D, TQ), BF16),
            pltpu.VMEM((D, D), BF16),
            pltpu.VMEM((DH, D), BF16),
            pltpu.VMEM((DH, D), BF16),
            pltpu.VMEM((D, D), BF16),
            pltpu.VMEM((D, FF), BF16),
            pltpu.VMEM((D, FF), BF16),
            pltpu.VMEM((D, FF), BF16),
            pltpu.VMEM((1, D), BF16),
            pltpu.VMEM((D, 6 * D), BF16),
            pltpu.SemaphoreType.DMA((10,)),
            pltpu.SemaphoreType.DMA((NQB,)),
            pltpu.SemaphoreType.DMA((NQB,)),
            pltpu.VMEM((6 * D, 128), F32),
            pltpu.VMEM((NQKV, D), BF16),
            pltpu.VMEM((D, D), BF16),
            pltpu.VMEM((HPI, S, KW), BF16),
            pltpu.VMEM((VR, S), F32),
            pltpu.VMEM((NQB, D, TQ), F32),
            pltpu.VMEM((2, S, TQ), F32),
            pltpu.VMEM((2, 1, TQ), F32),
            pltpu.VMEM((NQB, D, TQ), F32),
            pltpu.VMEM((NQB, D, TQ), F32),
            pltpu.VMEM((NQB, TQ, D), BF16),
            pltpu.VMEM((NQB, D, TQ), F32),
            pltpu.VMEM((NQB, D, TQ), BF16),
        ],
        compiler_params=pltpu.CompilerParams(vmem_limit_bytes=100 * 1024 * 1024),
    )(
        jnp.transpose(A_x, (0, 2, 1)), A_wq, A_wk.T, A_wv.T, A_wo,
        B_w_gate, B_w_up, B_w_down.T, c, w_mod,
    )
    return jnp.transpose(out_t, (0, 2, 1))
```

```python
import math

import jax
import jax.numpy as jnp
import jax.experimental.pallas as pl
import jax.experimental.pallas.tpu as pltpu

F32 = jnp.float32
BF16 = jnp.bfloat16

S = 2048
D = 576
H = 32
DH = D // H
FF = 4608
EPS = 1e-05

KW = 24
VR = 24
NKV = 2 * KW
NQKV = NKV + D

TA = 256
NA = S // TA
TQ = 512
NQB = S // TQ
KC = 128
NCH = S // KC
HPI = 8
IPB = H // HPI
LAG = 2
NT = NQB * H
TM = 256
NM = S // TM
FC = 768
NFH = 2
FH = FF // NFH
DPB = NFH * TQ // TM
MOD1 = 2 * D

NV = 240
VB = 16
PRE = 2
SM = S - NV
_base = (SM // NCH) // 16 * 16
_extra = (SM - _base * NCH) // 16
QK_SIZES = [_base + (16 if (i * _extra) // NCH != ((i + 1) * _extra) // NCH else 0) for i in range(NCH)]
QK_OFFS = [sum(QK_SIZES[:i]) for i in range(NCH)]
assert sum(QK_SIZES) == SM and NV <= TA

QK_SCALE = (DH ** -0.5) * math.log2(math.e)


def _dot(a, b):
    return jnp.dot(a, b, preferred_element_type=F32)


def _dot_nt(a, b):
    return jax.lax.dot_general(a, b, (((1,), (1,)), ((), ())), preferred_element_type=F32)


def _ln_t(x):
    m = jnp.mean(x, axis=0, keepdims=True)
    xc = x - m
    v = jnp.mean(xc * xc, axis=0, keepdims=True)
    return xc * jax.lax.rsqrt(v + EPS)


def _silu(g):
    h = 0.5 * g
    return h + h * jnp.tanh(h)


def _lanes(col, n):
    return jnp.concatenate([col] * (n // 128), axis=1)


def _rowmax8(s):
    return jnp.max(s.reshape(s.shape[0] // 8, 8, s.shape[1]), axis=0)


def _aligned(x, n):
    return x if isinstance(x, int) else pl.multiple_of(x, n)


def _kernel(
    xt_hbm, wq_hbm, wkt_hbm, wvt_hbm, wo_hbm, wg_hbm, wu_hbm, wdt_hbm, c_hbm, wmod_hbm,
    out_hbm,
    xt_ref, wq_ref, wkt_ref, wvt_ref, wo_ref, wg_ref, wu_ref, wdt_ref, c_ref, wmod_ref,
    in_sems, x_sems, w_sems, out_sems,
    mod_ref, wqkv_ref, wot_ref, h1_ref, ks_ref, k0_ref, kb_ref, vt_ref, qt_ref,
    s_ref, m_ref, sv_ref, mv_ref, pacc_ref, pmax_ref, ot_ref,
    x1_ref, h2_ref, stage_ref,
):
    def copy(src, dst, sem):
        return pltpu.make_async_copy(src, dst, sem)

    cp_c = copy(c_hbm, c_ref, in_sems.at[0])
    cp_m1 = copy(wmod_hbm.at[:, pl.ds(0, MOD1)], wmod_ref.at[:, pl.ds(0, MOD1)], in_sems.at[1])
    cp_q = copy(wq_hbm, wq_ref, in_sems.at[2])
    cp_k = copy(wkt_hbm, wkt_ref, in_sems.at[3])
    cp_v = copy(wvt_hbm, wvt_ref, in_sems.at[4])
    cp_x = [copy(xt_hbm.at[0, :, pl.ds(i * TA, TA)], xt_ref.at[:, pl.ds(i * TA, TA)], x_sems.at[i])
            for i in range(NA)]
    cp_o = copy(wo_hbm, wo_ref, in_sems.at[5])
    cp_m2 = copy(wmod_hbm.at[:, pl.ds(MOD1, 6 * D - MOD1)], wmod_ref.at[:, pl.ds(MOD1, 6 * D - MOD1)],
                 in_sems.at[6])
    cp_w = [copy(w_hbm.at[:, pl.ds(fh * FH, FH)], w_ref.at[fh], w_sems.at[k * NFH + fh])
            for fh in range(NFH)
            for k, (w_hbm, w_ref) in enumerate(((wg_hbm, wg_ref), (wu_hbm, wu_ref), (wdt_hbm, wdt_ref)))]

    cp_q.start()
    cp_c.start()
    cp_k.start()
    cp_v.start()
    cp_m1.start()

    s_ref[1, (NCH - LAG) * KC - NV:SM, :] = jnp.zeros((LAG * KC, TQ), F32)
    pmax_ref[...] = jnp.zeros((1, TQ), F32)
    pacc_ref[...] = jnp.ones((VR, TQ), F32)

    cp_q.wait()
    cp_x[0].start()
    cp_x[1].start()
    wqkv_ref[NKV:NQKV, :] = wq_ref[...].astype(F32).T.astype(BF16)
    cp_k.wait()
    cp_v.wait()
    zpad = jnp.zeros((KW - DH, D), F32)
    kv_t = jnp.concatenate(
        [wkt_ref[...].astype(F32), zpad, wvt_ref[...].astype(F32), zpad], axis=0)
    wqkv_ref[0:NKV, :] = kv_t.astype(BF16)

    cp_c.wait()
    sc = jnp.broadcast_to(_silu(c_ref[...].astype(F32)), (8, D))

    def mod_cols(lo, hi):
        mod = _dot(sc, wmod_ref[:, lo:hi])
        mod_ref[lo:hi, :] = jnp.broadcast_to(mod[0:1, :], (128, hi - lo)).T

    cp_m1.wait()
    for i in range(2, NA):
        cp_x[i].start()
    mod_cols(0, MOD1)

    def ln1(i):
        tok = pl.ds(_aligned(i * TA, TA), TA)
        sa = _lanes(mod_ref[0:D, :], TA)
        ca1 = 1.0 + _lanes(mod_ref[D:2 * D, :], TA)
        x = xt_ref[:, tok].astype(F32)
        h1_ref[:, tok] = (_ln_t(x) * ca1 + sa).astype(BF16)

    def proj(i):
        tok = pl.ds(_aligned(i * TA, TA), TA)
        h = h1_ref[:, tok]
        kv = _dot(wqkv_ref[0:NKV, :], h)
        row = jax.lax.broadcasted_iota(jnp.int32, (VR, TA), 0)
        vt_ref[:, tok] = jnp.where(row == DH, 1.0, kv[KW:NKV, :])
        kt = jnp.concatenate(
            [kv[0:KW, :] * QK_SCALE, jnp.zeros((128 - KW, TA), F32)], axis=0)
        k = kt.T
        for r in range(4):
            kr = k if r == 0 else pltpu.roll(k, 2 * r, 1)
            ks_ref[r, tok, :] = kr[:, 0:KW].astype(BF16)
        if isinstance(i, int) and i == 0:
            k0_ref[...] = k
        qtok = pl.ds(_aligned((i % (TQ // TA)) * TA, TA), TA)
        qt_ref[i // (TQ // TA), :, qtok] = _dot(wqkv_ref[NKV:NQKV, :], h)

    def q_window(t4, r, lanes=slice(None)):
        base = _aligned((t4 % (H // 4)) * (4 * DH) + 16 * r, 8)
        return qt_ref[t4 // (H // 4), pl.ds(base, KW), lanes]

    def sv_mxu(g4):
        for r in range(4):
            base = _aligned(g4 * (4 * DH) + 16 * r, 8)
            s = _dot(ks_ref[r, 0:NV, :], qt_ref[0, pl.ds(base, KW), :])
            sv_ref[4 * g4 + r] = s
            mv_ref[4 * g4 + r] = _rowmax8(s)

    cp_x[0].wait()
    ln1(0)
    cp_x[1].wait()
    ln1(1)
    proj(0)
    for i in range(2, NA):
        cp_x[i].wait()
    cp_o.start()
    cp_m2.start()
    ln1(2)
    proj(1)
    for i in range(2, NA - 2):
        ln1(i + 1)
        proj(i)
        sv_mxu(i - 2)
    ln1(NA - 1)
    cp_o.wait()
    cp_m2.wait()
    for cp in cp_w:
        cp.start()
    proj(NA - 2)
    mod_cols(MOD1, 6 * D)
    proj(NA - 1)
    wot_ref[...] = wo_ref[...].astype(F32).T.astype(BF16)
    for g4 in range(NA - 4, H // 4):
        sv_mxu(g4)
    for d in range(DH):
        kb_ref[d] = jnp.broadcast_to(k0_ref[0:NV, d:d + 1], (NV, 128))

    def qk_chunk(q, r, slot, cidx, m):
        off, size = QK_OFFS[cidx], QK_SIZES[cidx]
        s = _dot(ks_ref[r, NV + off:NV + off + size, :], q)
        s_ref[slot, off:off + size, :] = s
        mc = _rowmax8(s)
        return mc if m is None else jnp.maximum(m, mc)

    def pv_chunk(slot, head, cidx, mp, acc):
        lo, hi = cidx * KC, (cidx + 1) * KC
        parts = []
        if lo < NV:
            parts.append(sv_ref[head, lo:min(hi, NV), :])
        if hi > NV:
            parts.append(s_ref[slot, max(lo, NV) - NV:hi - NV, :])
        s = parts[0] if len(parts) == 1 else jnp.concatenate(parts, axis=0)
        p = jnp.exp2(s - mp).astype(BF16)
        o = _dot(vt_ref[:, lo:hi], p)
        return o if acc is None else acc + o

    def store_o(g4, r, acc):
        ot_ref[g4, r * DH:(r + 1) * DH, :] = acc[0:DH, :] * (1.0 / acc[DH:DH + 1, :])

    q0 = q_window(0, 0)
    m = None
    for cidx in range(NCH):
        m = qk_chunk(q0, 0, 0, cidx, m)
    m_ref[0] = m

    def attn_block(it):
        t4 = it * (HPI // 4)
        h0 = (it % IPB) * HPI
        m = None
        q = None
        acc = pacc_ref[...]
        mp = pmax_ref[...]
        for t in range(HPI * NCH):
            u, cidx = divmod(t, NCH)
            hq = u + 1
            if cidx == 0:
                tq4 = t4 + hq // 4
                if hq == HPI:
                    tq4 = jnp.minimum(tq4, NT // 4 - 1)
                q = q_window(tq4, hq % 4)
                m = None
            m = qk_chunk(q, hq % 4, hq % 2, cidx, m)
            if cidx == NCH - 1:
                m_ref[hq % 2] = m
            up, cp = divmod(t - LAG, NCH)
            if cp == 0:
                acc = None
                mp = jnp.max(jnp.maximum(m_ref[up % 2], mv_ref[h0 + up]), axis=0, keepdims=True)
            acc = pv_chunk(up % 2, h0 + up, cp, mp, acc)
            if cp == NCH - 1:
                g4 = t4 + up // 4
                if up < 0 and not isinstance(g4, int):
                    g4 = jnp.maximum(g4, 0)
                store_o(g4, up % 4, acc)
        pacc_ref[...] = acc
        pmax_ref[...] = mp

    def c1(mb):
        tok = pl.ds(_aligned(mb * TM, TM), TM)
        qb = mb // (TQ // TM)
        qtok = pl.ds(_aligned((mb % (TQ // TM)) * TM, TM), TM)
        ga = _lanes(mod_ref[2 * D:3 * D, :], TM)
        o = ot_ref[pl.ds(qb * (H // 4), H // 4), :, qtok].reshape(D, TM)
        x1_ref[mb] = xt_ref[:, tok].astype(F32) + ga * _dot(wot_ref[...], o)

    def c2(mb, dst, lo, n):
        tok = pl.ds(_aligned(lo, 128), n)
        sb = _lanes(mod_ref[3 * D:4 * D, :], n)
        cb1 = 1.0 + _lanes(mod_ref[4 * D:5 * D, :], n)
        h2_ref[dst, tok, :] = (_ln_t(x1_ref[mb, :, tok]) * cb1 + sb).T.astype(BF16)

    def finish_block(qb):
        acc = pacc_ref[...]
        mp = pmax_ref[...]
        for cp in range(NCH - LAG, NCH):
            acc = pv_chunk(1, H - 1, cp, mp, acc)
        store_o(qb * (H // 4) + H // 4 - 1, 3, acc)
        c1(2 * qb)
        c1(2 * qb + 1)
        c2(2 * qb, 2 * qb, 0, TM)

    def out_copy(mb):
        return copy(stage_ref.at[mb], out_hbm.at[0, :, pl.ds(_aligned(mb * TM, TM), TM)],
                    out_sems.at[mb])

    def vpu_scores(i):
        zero = jax.lax.shift_right_logical(i, 16)
        qb_next = jnp.minimum(i // DPB + 1, NQB - 1)
        t4base = qb_next * (H // 4) + (i % DPB) * (H // 4 // DPB)

        def unit(t4, r, j, prev):
            head = (t4 % (H // 4)) * 4 + r
            lanes = pl.ds(_aligned(j * 128, 128), 128)
            qw = q_window(t4, r, lanes)
            qd = [jnp.broadcast_to(qw[2 * r + d:2 * r + d + 1, :], (VB, 128)) for d in range(DH)]
            m = None
            for kb in range(NV // VB):
                terms = [kb_ref[d, kb * VB:(kb + 1) * VB, :] * qd[d] for d in range(DH)]
                terms = ([terms[2 * i] + terms[2 * i + 1] for i in range(PRE)] + terms[2 * PRE:])
                sv = pltpu.bitcast(pltpu.bitcast(prev, jnp.int32) & zero, F32)
                for x in terms:
                    sv = sv + x
                prev = sv
                sv_ref[head, kb * VB:(kb + 1) * VB, lanes] = sv
                mc = _rowmax8(sv)
                m = mc if m is None else jnp.maximum(m, mc)
            mv_ref[head, :, lanes] = m
            return prev

        def step(n, prev):
            for r in range(4):
                prev = unit(t4base + n // 4, r, n % 4, prev)
            return prev

        jax.lax.fori_loop(0, H // DPB, step, jnp.zeros((VB, 128), F32), unroll=True)

    def ffn(i, carry):
        mb = i // NFH
        fh = i % NFH
        h = h2_ref[mb]
        vpu_scores(i)
        acc = None
        for fc in range(FH // FC):
            cols = slice(fc * FC, (fc + 1) * FC)
            g = _dot(h, wg_ref[fh, :, cols])
            u = _dot(h, wu_ref[fh, :, cols])
            a = (_silu(g) * u).astype(BF16)
            y = _dot_nt(wdt_ref[fh, :, cols], a)
            acc = y if acc is None else acc + y
        c2(mb | 1, jnp.where(mb % 2 == 0, mb + 1, NM), fh * (TM // NFH), TM // NFH)
        gb = _lanes(mod_ref[5 * D:6 * D, :], TM)
        x2 = x1_ref[mb] + gb * acc
        x1_ref[mb] = x2
        stage_ref[mb] = x2.astype(BF16)

        @pl.when(fh == NFH - 1)
        def _():
            out_copy(mb).start()

        return carry

    def main_loop(it, carry):
        attn_block(it)

        @pl.when(it % IPB == IPB - 1)
        def _():
            @pl.when(it == IPB - 1)
            def _():
                for cp in cp_w:
                    cp.wait()

            qb = it // IPB
            finish_block(qb)
            jax.lax.fori_loop(qb * DPB, (qb + 1) * DPB, ffn, 0)

        return carry

    jax.lax.fori_loop(0, NT // HPI, main_loop, 0)
    for mb in range(NM):
        out_copy(mb).wait()


@jax.jit
def pallas_adaLN_cond__grouped_kv_mqa__swiglu_ffn__prompt_kernel(
    A_x: jax.Array,
    A_wq: jax.Array,
    A_wk: jax.Array,
    A_wv: jax.Array,
    A_wo: jax.Array,
    B_x: jax.Array,
    B_w_gate: jax.Array,
    B_w_up: jax.Array,
    B_w_down: jax.Array,
    c: jax.Array,
    w_mod: jax.Array,
):
    del B_x
    hbm = pl.BlockSpec(memory_space=pltpu.HBM)
    out_t = pl.pallas_call(
        _kernel,
        out_shape=jax.ShapeDtypeStruct((1, D, S), A_x.dtype),
        in_specs=[hbm] * 10,
        out_specs=hbm,
        scratch_shapes=[
            pltpu.VMEM((D, S), BF16),
            pltpu.VMEM((D, D), BF16),
            pltpu.VMEM((DH, D), BF16),
            pltpu.VMEM((DH, D), BF16),
            pltpu.VMEM((D, D), BF16),
            pltpu.VMEM((NFH, D, FH), BF16),
            pltpu.VMEM((NFH, D, FH), BF16),
            pltpu.VMEM((NFH, D, FH), BF16),
            pltpu.VMEM((1, D), BF16),
            pltpu.VMEM((D, 6 * D), BF16),
            pltpu.SemaphoreType.DMA((7,)),
            pltpu.SemaphoreType.DMA((NA,)),
            pltpu.SemaphoreType.DMA((3 * NFH,)),
            pltpu.SemaphoreType.DMA((NM,)),
            pltpu.VMEM((6 * D, 128), F32),
            pltpu.VMEM((NQKV, D), BF16),
            pltpu.VMEM((D, D), BF16),
            pltpu.VMEM((D, S), BF16),
            pltpu.VMEM((4, S, KW), BF16),
            pltpu.VMEM((TA, 128), F32),
            pltpu.VMEM((DH, NV, 128), F32),
            pltpu.VMEM((VR, S), F32),
            pltpu.VMEM((NQB, D, TQ), F32),
            pltpu.VMEM((2, SM, TQ), F32),
            pltpu.VMEM((2, 8, TQ), F32),
            pltpu.VMEM((H, NV, TQ), F32),
            pltpu.VMEM((H, 8, TQ), F32),
            pltpu.VMEM((VR, TQ), F32),
            pltpu.VMEM((1, TQ), F32),
            pltpu.VMEM((NT // 4, 4 * DH, TQ), F32),
            pltpu.VMEM((NM, D, TM), F32),
            pltpu.VMEM((NM + 1, TM, D), BF16),
            pltpu.VMEM((NM, D, TM), BF16),
        ],
        compiler_params=pltpu.CompilerParams(vmem_limit_bytes=100 * 1024 * 1024),
    )(
        jnp.transpose(A_x, (0, 2, 1)), A_wq, A_wk.T, A_wv.T, A_wo,
        B_w_gate, B_w_up, B_w_down.T, c, w_mod,
    )
    return jnp.transpose(out_t, (0, 2, 1))
```

```python
import math

import jax
import jax.numpy as jnp
import jax.experimental.pallas as pl
import jax.experimental.pallas.tpu as pltpu

F32 = jnp.float32
BF16 = jnp.bfloat16

S = 2048
D = 576
H = 32
DH = D // H
FF = 4608
EPS = 1e-05

KW = 24
VR = 24
NKV = 2 * KW
NQKV = NKV + D
ONE = (23, 23, 23, 0)

TM = 256
NM = S // TM
TQ = 512
NQB = S // TQ
NTL = TQ // 128
KC = 128
NCH = S // KC
HPI = 8
IPB = H // HPI
LAG = 3
RING = 8
NT = NQB * H
FC = 768
NFH = 2
FH = FF // NFH
DPB = NFH * TQ // TM
MOD1 = 2 * D

NV = 240
VB = 16
PRE = 2
NC = 208


def _tile_groups():
    gv, gc = NV // 16, NC // 16
    per = [((c + 1) * (gv + gc)) // NCH - (c * (gv + gc)) // NCH for c in range(NCH)]
    tail = sum(per[NCH - LAG:])
    kinds, a, b = [], 0, 0
    for _ in range(gv + gc - tail):
        if a < gv and (a * (gc - tail) <= b * gv or b >= gc - tail):
            kinds.append("v")
            a += 1
        else:
            kinds.append("c")
            b += 1
    kinds += ["c"] * tail
    tiles, i, idx = [], 0, {"v": 0, "c": 0}
    for c in range(NCH):
        tiles.append([])
        for _ in range(per[c]):
            tiles[c].append((kinds[i], idx[kinds[i]]))
            idx[kinds[i]] += 1
            i += 1
    assert idx == {"v": gv, "c": gc}
    return tiles


TILES = _tile_groups()
MSZ = [KC - 16 * len(t) for t in TILES]
MG0 = [sum(MSZ[:c]) // 8 for c in range(NCH)]
PIECES = [(j, kb) for j in range(NTL) for kb in range(NC // 8)]
PIECE_POS = [((pi + 1) * (sum(MSZ) // 8)) // len(PIECES) - 1 for pi in range(len(PIECES))]

QK_SCALE = (DH ** -0.5) * math.log2(math.e)
L_LO, L_HI = 2.0 ** -64, 2.0 ** 64


def _dot(a, b):
    return jnp.dot(a, b, preferred_element_type=F32)


def _dot_nt(a, b):
    return jax.lax.dot_general(a, b, (((1,), (1,)), ((), ())), preferred_element_type=F32)


def _ln_t(x):
    m = jnp.mean(x, axis=0, keepdims=True)
    xc = x - m
    v = jnp.mean(xc * xc, axis=0, keepdims=True)
    return xc * jax.lax.rsqrt(v + EPS)


def _silu(g):
    h = 0.5 * g
    return h + h * jnp.tanh(h)


def _lanes(col, n):
    return jnp.concatenate([col] * (n // 128), axis=1)


def _rowmax8(s):
    return jnp.max(s.reshape(s.shape[0] // 8, 8, s.shape[1]), axis=0)


def _aligned(x, n):
    return x if isinstance(x, int) else pl.multiple_of(x, n)


def _tie(x, zero):
    return pltpu.bitcast(pltpu.bitcast(x, jnp.int32) & zero, F32)


def _kernel(
    xt_hbm, wq_hbm, wkt_hbm, wvt_hbm, wo_hbm, wg_hbm, wu_hbm, wdt_hbm, c_hbm, wmod_hbm,
    out_hbm,
    xt_ref, wq_ref, wkv_ref, wo_ref, wg_ref, wu_ref, wdt_ref, c_ref, wmod_ref,
    in_sems, x_sems, w_sems, out_sems,
    mod_ref, wqkv_ref, wot_ref, h1_ref, ks_ref, ksp_ref, k0_ref, kb_ref, vt_ref, qt_ref,
    s_ref, sv_ref, mv_ref, sb_ref, pacc_ref, pneg_ref, bad_ref, ot_ref,
    x1_ref, h2_ref, stage_ref,
):
    def copy(src, dst, sem):
        return pltpu.make_async_copy(src, dst, sem)

    cp_c = copy(c_hbm, c_ref.at[0], in_sems.at[0])
    cp_m1 = copy(wmod_hbm.at[:, pl.ds(0, MOD1)], wmod_ref.at[:, pl.ds(0, MOD1)], in_sems.at[1])
    cp_q = copy(wq_hbm, wq_ref, in_sems.at[2])
    cp_k = copy(wkt_hbm, wkv_ref.at[0], in_sems.at[3])
    cp_v = copy(wvt_hbm, wkv_ref.at[1], in_sems.at[4])
    cp_x = [copy(xt_hbm.at[0, :, pl.ds(i * TM, TM)], xt_ref.at[i], x_sems.at[i]) for i in range(NM)]
    cp_o = copy(wo_hbm, wo_ref, in_sems.at[5])
    cp_m2 = copy(wmod_hbm.at[:, pl.ds(MOD1, 6 * D - MOD1)], wmod_ref.at[:, pl.ds(MOD1, 6 * D - MOD1)],
                 in_sems.at[6])
    cp_w = [copy(w_hbm.at[:, pl.ds(fh * FH, FH)], w_ref.at[fh], w_sems.at[k * NFH + fh])
            for fh in range(NFH)
            for k, (w_hbm, w_ref) in enumerate(((wg_hbm, wg_ref), (wu_hbm, wu_ref), (wdt_hbm, wdt_ref)))]

    cp_q.start()
    cp_c.start()
    cp_k.start()
    cp_v.start()
    cp_m1.start()

    for cidx in range(NCH - LAG, NCH):
        s_ref[cidx % RING] = jnp.zeros((KC, TQ), F32)
        for _, g in TILES[cidx]:
            sb_ref[3, g * 16:(g + 1) * 16, :] = jnp.zeros((16, TQ), F32)
    pneg_ref[...] = jnp.zeros((8, TQ), F32)
    pacc_ref[...] = jnp.ones((VR, TQ), F32)
    bad_ref[...] = jnp.zeros((8, TQ), F32)

    cp_q.wait()
    cp_x[0].start()
    cp_x[1].start()
    wqkv_ref[NKV:NQKV, :] = wq_ref[...].astype(F32).T.astype(BF16)
    cp_k.wait()
    cp_v.wait()
    zpad = jnp.zeros((KW - DH, D), F32)
    kv_t = jnp.concatenate(
        [wkv_ref[0].astype(F32), zpad, wkv_ref[1].astype(F32), zpad], axis=0)
    wqkv_ref[0:NKV, :] = kv_t.astype(BF16)

    cp_c.wait()
    sc = jnp.broadcast_to(_silu(c_ref[0].astype(F32)), (8, D))

    def mod_cols(lo, hi):
        mod = _dot(sc, wmod_ref[:, lo:hi])
        mod_ref[lo:hi, :] = jnp.broadcast_to(mod[0:1, :], (128, hi - lo)).T

    cp_m1.wait()
    for i in range(2, NM):
        cp_x[i].start()
    mod_cols(0, MOD1)

    def ln1(i):
        sa = _lanes(mod_ref[0:D, :], TM)
        ca1 = 1.0 + _lanes(mod_ref[D:2 * D, :], TM)
        h1_ref[i] = (_ln_t(xt_ref[i].astype(F32)) * ca1 + sa).astype(BF16)

    def proj(i):
        tok = slice(i * TM, (i + 1) * TM)
        h = h1_ref[i]
        kv = _dot(wqkv_ref[0:NKV, :], h)
        row = jax.lax.broadcasted_iota(jnp.int32, (VR, TM), 0)
        vt_ref[:, tok] = jnp.where(row == DH, 1.0, kv[KW:NKV, :])
        kt = jnp.concatenate(
            [kv[0:KW, :] * QK_SCALE, jnp.zeros((128 - KW, TM), F32)], axis=0)
        k = kt.T
        lane = jax.lax.broadcasted_iota(jnp.int32, (TM, 128), 1)
        packed = []
        for cidx in range(i * TM // KC, (i + 1) * TM // KC):
            for n, (kind, g) in enumerate(TILES[cidx]):
                packed.append((cidx * KC - i * TM + MSZ[cidx] + 16 * n,
                               16 * g + (0 if kind == "v" else NV)))
        for r in range(4):
            kr = k if r == 0 else pltpu.roll(k, 2 * r, 1)
            kr = jnp.where(lane == ONE[r], 1.0, kr)[:, 0:KW].astype(BF16)
            ks_ref[r, tok, :] = kr
            for src, dst in packed:
                if dst < NV or r == 0:
                    ksp_ref[r, dst:dst + 16, :] = kr[src:src + 16, :]
        for src, dst in packed:
            k0_ref[dst:dst + 16, :] = k[src:src + 16, :]
        qb, off = divmod(i * TM, TQ)
        qt_ref[qb, :, off:off + TM] = _dot(wqkv_ref[NKV:NQKV, :], h)

    def q_window(t4, r, lanes=slice(None)):
        base = _aligned((t4 % (H // 4)) * (4 * DH) + 16 * r, 8)
        return qt_ref[t4 // (H // 4), pl.ds(base, KW), lanes]

    wrow = jax.lax.broadcasted_iota(jnp.int32, (KW, TQ), 0)

    def sv_mxu(g4):
        for r in range(4):
            s = _dot(ksp_ref[r, 0:NV, :], jnp.where(wrow == ONE[r], 0.0, q_window(g4, r)))
            sv_ref[4 * g4 + r] = s
            mv_ref[4 * g4 + r] = _rowmax8(s)

    cp_x[0].wait()
    ln1(0)
    cp_x[1].wait()
    ln1(1)
    proj(0)
    for i in range(2, NM):
        cp_x[i].wait()
    cp_o.start()
    cp_m2.start()
    for i in range(1, NM - 1):
        ln1(i + 1)
        proj(i)
    cp_o.wait()
    cp_m2.wait()
    for cp in cp_w:
        cp.start()
    proj(NM - 1)
    mod_cols(MOD1, 6 * D)
    wot_ref[...] = wo_ref[...].astype(F32).T.astype(BF16)
    for g4 in range(H // 4):
        sv_mxu(g4)
    sb_ref[0] = _dot(ksp_ref[0, NV:NV + NC, :], jnp.where(wrow == ONE[0], 0.0, q_window(0, 0)))
    for d in range(DH):
        kb_ref[d] = jnp.broadcast_to(k0_ref[:, d:d + 1], (NV + NC, 128))

    def pv_tile(hs, cidx):
        parts = [s_ref[cidx % RING, 0:MSZ[cidx], :]]
        neg16 = jnp.concatenate([hs["neg"], hs["neg"]], axis=0)
        for kind, g in TILES[cidx]:
            rows = slice(g * 16, (g + 1) * 16)
            raw = sv_ref[hs["head"], rows, :] if kind == "v" else sb_ref[hs["u"] % 4, rows, :]
            parts.append(raw + neg16)
        p = jnp.exp2(jnp.concatenate(parts, axis=0)).astype(BF16)
        o = _dot(vt_ref[:, cidx * KC:(cidx + 1) * KC], p)
        hs["acc"] = o if hs["acc"] is None else hs["acc"] + o

    def store_o(g4, r, acc):
        ot_ref[g4, r * DH:(r + 1) * DH, :] = acc[0:DH, :] * (1.0 / acc[DH:DH + 1, :])

    def flag(acc, bad):
        l = acc[16:24, :]
        ok = jnp.logical_and(l >= L_LO, l <= L_HI)
        row8 = jax.lax.broadcasted_iota(jnp.int32, (8, TQ), 0)
        return jnp.where(jnp.logical_or(ok, row8 != DH - 16), bad, 1.0)

    def attn_block(it):
        zero = jax.lax.shift_right_logical(it, 16)
        t4 = it * (HPI // 4)
        h0 = (it % IPB) * HPI
        bad = bad_ref[...]
        hs = {"acc": pacc_ref[...], "u": -1, "head": None, "neg": pneg_ref[...]}
        pend = [(hs, cidx) for cidx in range(NCH - LAG, NCH)]
        for u in range(HPI):
            r = u % 4
            mx = jnp.max(mv_ref[h0 + u], axis=0, keepdims=True)
            neg = jnp.broadcast_to(-mx, (8, TQ))
            neg = pltpu.bitcast(pltpu.bitcast(neg, jnp.int32) & jnp.int32(-65536), F32)
            q = jnp.where(wrow == ONE[r], jnp.concatenate([neg] * (KW // 8), axis=0),
                          q_window(t4 + u // 4, r))
            hs = {"acc": None, "u": u, "head": h0 + u, "neg": neg}
            rn = (u + 1) % 4
            tn4 = t4 + (u + 1) // 4
            if u == HPI - 1:
                tn4 = jnp.minimum(tn4, NT // 4 - 1)
            for cidx in range(NCH):
                s = _dot(ks_ref[r, cidx * KC:cidx * KC + MSZ[cidx], :], q)
                s_ref[cidx % RING, 0:MSZ[cidx], :] = s
                for pi, (j, kb) in enumerate(PIECES):
                    if not MG0[cidx] <= PIECE_POS[pi] < MG0[cidx] + MSZ[cidx] // 8:
                        continue
                    if kb == 0:
                        qw = q_window(tn4, rn, slice(j * 128, (j + 1) * 128))
                        qd = jnp.stack([
                            jnp.broadcast_to(qw[2 * rn + d:2 * rn + d + 1, :], (8, 128))
                            for d in range(DH)])
                    sv = jnp.sum(kb_ref[:, NV + kb * 8:NV + (kb + 1) * 8, :] * qd, axis=0)
                    ar = (PIECE_POS[pi] - MG0[cidx]) * 8
                    sv = sv + _tie(s[ar:ar + 8, (pi % NTL) * 128:(pi % NTL + 1) * 128], zero)
                    sb_ref[rn, kb * 8:(kb + 1) * 8, j * 128:(j + 1) * 128] = sv
                pend.append((hs, cidx))
                hp, cp = pend.pop(0)
                pv_tile(hp, cp)
                if cp == NCH - 1:
                    g4 = t4 + hp["u"] // 4
                    if hp["u"] < 0:
                        g4 = jnp.maximum(g4, 0)
                    store_o(g4, hp["u"] % 4, hp["acc"])
                    bad = flag(hp["acc"], bad)
        pacc_ref[...] = hs["acc"]
        pneg_ref[...] = hs["neg"]
        bad_ref[...] = bad

    def attn_exact(qb):
        def head(h, carry):
            r = h % 4
            base = pl.multiple_of((h // 4) * (4 * DH) + 16 * r, 8)
            one = jnp.where(r == 3, ONE[3], ONE[0])
            q = jnp.where(wrow == one, 0.0, qt_ref[qb, pl.ds(base, KW), :])

            def scores(cidx):
                return _dot(ks_ref[r, pl.ds(pl.multiple_of(cidx * KC, KC), KC), :], q)

            m = jax.lax.fori_loop(
                0, NCH, lambda cidx, m: jnp.maximum(m, _rowmax8(scores(cidx))),
                jnp.full((8, TQ), -jnp.inf, F32))
            m = jnp.max(m, axis=0, keepdims=True)

            def pv(cidx, acc):
                p = jnp.exp2(scores(cidx) - m).astype(BF16)
                return acc + _dot(vt_ref[:, pl.ds(pl.multiple_of(cidx * KC, KC), KC)], p)

            acc = jax.lax.fori_loop(0, NCH, pv, jnp.zeros((VR, TQ), F32))
            for rr in range(4):
                @pl.when(r == rr)
                def _():
                    store_o(qb * (H // 4) + h // 4, rr, acc)
            return carry

        jax.lax.fori_loop(0, H, head, 0)

    def c1(qb, half):
        mb = 2 * qb + half
        ga = _lanes(mod_ref[2 * D:3 * D, :], TM)
        o = ot_ref[pl.ds(qb * (H // 4), H // 4), :, half * TM:(half + 1) * TM].reshape(D, TM)
        x1 = xt_ref[mb].astype(F32) + ga * _dot(wot_ref[...], o)
        for e in range(NFH):
            x1_ref[NFH * mb + e] = x1[:, e * 128:(e + 1) * 128]

    def c2(src, dst):
        sb = mod_ref[3 * D:4 * D, :]
        cb1 = 1.0 + mod_ref[4 * D:5 * D, :]
        h2_ref[dst] = (_ln_t(x1_ref[src]) * cb1 + sb).T.astype(BF16)

    def finish_block(qb):
        hs = {"acc": pacc_ref[...], "u": -1, "head": None, "neg": pneg_ref[...]}
        for cidx in range(NCH - LAG, NCH):
            pv_tile(hs, cidx)
        store_o(qb * (H // 4) + H // 4 - 1, 3, hs["acc"])
        bad = jnp.max(flag(hs["acc"], bad_ref[...]))
        bad_ref[...] = jnp.zeros((8, TQ), F32)

        @pl.when(bad > 0.0)
        def _():
            attn_exact(qb)

        c1(qb, 0)
        c1(qb, 1)
        for e in range(NFH):
            c2(DPB * qb + e, DPB * qb + e)

    def out_copy(mb):
        return copy(stage_ref.at[mb], out_hbm.at[0, :, pl.ds(_aligned(mb * TM, TM), TM)],
                    out_sems.at[mb])

    def vpu_scores(i):
        zero = jax.lax.shift_right_logical(i, 16)
        qb_next = jnp.minimum(i // DPB + 1, NQB - 1)
        t4base = qb_next * (H // 4) + (i % DPB) * (H // 4 // DPB)

        def unit(t4, r, j, prev):
            head = (t4 % (H // 4)) * 4 + r
            lanes = pl.ds(_aligned(j * 128, 128), 128)
            qw = q_window(t4, r, lanes)
            qd = [jnp.broadcast_to(qw[2 * r + d:2 * r + d + 1, :], (VB, 128)) for d in range(DH)]
            m = None
            for kb in range(NV // VB):
                terms = [kb_ref[d, kb * VB:(kb + 1) * VB, :] * qd[d] for d in range(DH)]
                terms = ([terms[2 * i] + terms[2 * i + 1] for i in range(PRE)] + terms[2 * PRE:])
                sv = _tie(prev, zero)
                for x in terms:
                    sv = sv + x
                prev = sv
                sv_ref[head, kb * VB:(kb + 1) * VB, lanes] = sv
                mc = _rowmax8(sv)
                m = mc if m is None else jnp.maximum(m, mc)
            mv_ref[head, :, lanes] = m
            return prev

        def step(n, prev):
            for r in range(4):
                prev = unit(t4base + n // 4, r, n % 4, prev)
            return prev

        jax.lax.fori_loop(0, H // DPB, step, jnp.zeros((VB, 128), F32), unroll=True)

    def ffn(i, carry):
        mb = i // NFH
        fh = i % NFH
        h = h2_ref[pl.ds(NFH * mb, NFH)].reshape(TM, D)
        vpu_scores(i)
        acc = None
        for fc in range(FH // FC):
            cols = slice(fc * FC, (fc + 1) * FC)
            g = _dot(h, wg_ref[fh, :, cols])
            u = _dot(h, wu_ref[fh, :, cols])
            a = (_silu(g) * u).astype(BF16)
            y = _dot_nt(wdt_ref[fh, :, cols], a)
            acc = y if acc is None else acc + y
        src = NFH * (mb | 1) + fh
        c2(src, jnp.where(mb % 2 == 0, src, NFH * NM))
        gb = mod_ref[5 * D:6 * D, :]
        for e in range(NFH):
            x2 = x1_ref[NFH * mb + e] + gb * acc[:, e * 128:(e + 1) * 128]
            x1_ref[NFH * mb + e] = x2
            stage_ref[mb, :, e * 128:(e + 1) * 128] = x2.astype(BF16)

        @pl.when(fh == NFH - 1)
        def _():
            out_copy(mb).start()

        return carry

    def main_loop(it, carry):
        attn_block(it)

        @pl.when(it % IPB == IPB - 1)
        def _():
            @pl.when(it == IPB - 1)
            def _():
                for cp in cp_w:
                    cp.wait()

            qb = it // IPB
            finish_block(qb)
            jax.lax.fori_loop(qb * DPB, (qb + 1) * DPB, ffn, 0)

        return carry

    jax.lax.fori_loop(0, NT // HPI, main_loop, 0)
    for mb in range(NM):
        out_copy(mb).wait()


@jax.jit
def pallas_adaLN_cond__grouped_kv_mqa__swiglu_ffn__prompt_kernel(
    A_x: jax.Array,
    A_wq: jax.Array,
    A_wk: jax.Array,
    A_wv: jax.Array,
    A_wo: jax.Array,
    B_x: jax.Array,
    B_w_gate: jax.Array,
    B_w_up: jax.Array,
    B_w_down: jax.Array,
    c: jax.Array,
    w_mod: jax.Array,
):
    del B_x
    hbm = pl.BlockSpec(memory_space=pltpu.HBM)
    out_t = pl.pallas_call(
        _kernel,
        out_shape=jax.ShapeDtypeStruct((1, D, S), A_x.dtype),
        in_specs=[hbm] * 10,
        out_specs=hbm,
        scratch_shapes=[
            pltpu.VMEM((NM, D, TM), BF16),
            pltpu.VMEM((D, D), BF16),
            pltpu.VMEM((8, DH, D), BF16),
            pltpu.VMEM((D, D), BF16),
            pltpu.VMEM((NFH, D, FH), BF16),
            pltpu.VMEM((NFH, D, FH), BF16),
            pltpu.VMEM((NFH, D, FH), BF16),
            pltpu.VMEM((32, 1, D), BF16),
            pltpu.VMEM((D, 6 * D), BF16),
            pltpu.SemaphoreType.DMA((7,)),
            pltpu.SemaphoreType.DMA((NM,)),
            pltpu.SemaphoreType.DMA((3 * NFH,)),
            pltpu.SemaphoreType.DMA((NM,)),
            pltpu.VMEM((6 * D, 128), F32),
            pltpu.VMEM((640, D), BF16),
            pltpu.VMEM((D, D), BF16),
            pltpu.VMEM((NM, D, TM), BF16),
            pltpu.VMEM((4, S, KW), BF16),
            pltpu.VMEM((4, NV + NC, KW), BF16),
            pltpu.VMEM((NV + NC, 128), F32),
            pltpu.VMEM((DH, NV + NC, 128), F32),
            pltpu.VMEM((VR, S), F32),
            pltpu.VMEM((NQB, D, TQ), F32),
            pltpu.VMEM((RING, KC, TQ), F32),
            pltpu.VMEM((H, NV, TQ), F32),
            pltpu.VMEM((H, 8, TQ), F32),
            pltpu.VMEM((4, NC, TQ), F32),
            pltpu.VMEM((VR, TQ), F32),
            pltpu.VMEM((8, TQ), F32),
            pltpu.VMEM((8, TQ), F32),
            pltpu.VMEM((NT // 4, 4 * DH, TQ), F32),
            pltpu.VMEM((NFH * NM, D, 128), F32),
            pltpu.VMEM((NFH * NM + 1, 128, D), BF16),
            pltpu.VMEM((NM, D, TM), BF16),
        ],
        compiler_params=pltpu.CompilerParams(
            vmem_limit_bytes=100 * 1024 * 1024, internal_scratch_in_bytes=65536),
    )(
        jnp.transpose(A_x, (0, 2, 1)), A_wq, A_wk.T, A_wv.T, A_wo,
        B_w_gate, B_w_up, B_w_down.T, c, w_mod,
    )
    return jnp.transpose(out_t, (0, 2, 1))
```

```python
import math

import jax
import jax.numpy as jnp
import jax.experimental.pallas as pl
import jax.experimental.pallas.tpu as pltpu

F32 = jnp.float32
BF16 = jnp.bfloat16

S = 2048
D = 576
H = 32
DH = D // H
FF = 4608
EPS = 1e-05

KW = 24
VR = 24
NKV = 2 * KW
NQKV = NKV + D
ONE = (23, 23, 23, 0)

TM = 256
NM = S // TM
TQ = 512
NQB = S // TQ
NTL = TQ // 128
KC = 128
NCH = S // KC
HPI = 8
IPB = H // HPI
LAG = 3
RING = 8
NT = NQB * H
FU = 256
WS = 0.8
NFH = 2
FH = FF // NFH
DPB = NFH * TQ // TM
MOD1 = 2 * D

NV = 288
NMX = 8
NC = 192


def _tile_groups():
    gv, gc = NV // 16, NC // 16
    per = [((c + 1) * (gv + gc)) // NCH - (c * (gv + gc)) // NCH for c in range(NCH)]
    tail = sum(per[NCH - LAG:])
    kinds, a, b = [], 0, 0
    for _ in range(gv + gc - tail):
        if a < gv and (a * (gc - tail) <= b * gv or b >= gc - tail):
            kinds.append("v")
            a += 1
        else:
            kinds.append("c")
            b += 1
    kinds += ["c"] * tail
    tiles, i, idx = [], 0, {"v": 0, "c": 0}
    for c in range(NCH):
        tiles.append([])
        for _ in range(per[c]):
            tiles[c].append((kinds[i], idx[kinds[i]]))
            idx[kinds[i]] += 1
            i += 1
    assert idx == {"v": gv, "c": gc}
    return tiles


TILES = _tile_groups()
MSZ = [KC - 16 * len(t) for t in TILES]
MG0 = [sum(MSZ[:c]) // 8 for c in range(NCH)]
PIECES = [(j, kb) for j in range(NTL) for kb in range(NC // 8)]
PIECE_POS = [((pi + 1) * (sum(MSZ) // 8)) // len(PIECES) - 1 for pi in range(len(PIECES))]

QK_SCALE = (DH ** -0.5) * math.log2(math.e)
L_LO, L_HI = 2.0 ** -64, 2.0 ** 64


def _dot(a, b):
    return jnp.dot(a, b, preferred_element_type=F32)


def _dot_nt(a, b):
    return jax.lax.dot_general(a, b, (((1,), (1,)), ((), ())), preferred_element_type=F32)


def _ln_t(x):
    m = jnp.mean(x, axis=0, keepdims=True)
    xc = x - m
    v = jnp.mean(xc * xc, axis=0, keepdims=True)
    return xc * jax.lax.rsqrt(v + EPS)


def _silu(g):
    h = 0.5 * g
    return h + h * jnp.tanh(h)


def _lanes(col, n):
    return jnp.concatenate([col] * (n // 128), axis=1)


def _rowmax8(s):
    return jnp.max(s.reshape(s.shape[0] // 8, 8, s.shape[1]), axis=0)


def _aligned(x, n):
    return x if isinstance(x, int) else pl.multiple_of(x, n)


def _tie(x, zero):
    return pltpu.bitcast(pltpu.bitcast(x, jnp.int32) & zero, F32)


def _kernel(
    xt_hbm, wq_hbm, wkt_hbm, wvt_hbm, wo_hbm, wg_hbm, wu_hbm, wdt_hbm, c_hbm, wmod_hbm,
    out_hbm,
    xt_ref, wq_ref, wkv_ref, wo_ref, wg_ref, wu_ref, wdt_ref, c_ref, wmod_ref,
    in_sems, x_sems, w_sems, out_sems,
    mod_ref, wqkv_ref, wot_ref, h1_ref, ks_ref, ksp_ref, k0_ref, kb_ref, vt_ref, qt_ref,
    s_ref, sv_ref, mv_ref, sb_ref, pacc_ref, pneg_ref, bad_ref, ot_ref,
    x1_ref, h2_ref, stage_ref,
):
    def copy(src, dst, sem):
        return pltpu.make_async_copy(src, dst, sem)

    cp_c = copy(c_hbm, c_ref.at[0], in_sems.at[0])
    cp_m1 = copy(wmod_hbm.at[:, pl.ds(0, MOD1)], wmod_ref.at[:, pl.ds(0, MOD1)], in_sems.at[1])
    cp_q = copy(wq_hbm, wq_ref, in_sems.at[2])
    cp_k = copy(wkt_hbm, wkv_ref.at[0], in_sems.at[3])
    cp_v = copy(wvt_hbm, wkv_ref.at[1], in_sems.at[4])
    cp_x = [copy(xt_hbm.at[0, :, pl.ds(i * TM, TM)], xt_ref.at[i], x_sems.at[i]) for i in range(NM)]
    cp_o = copy(wo_hbm, wo_ref, in_sems.at[5])
    cp_m2 = copy(wmod_hbm.at[:, pl.ds(MOD1, 6 * D - MOD1)], wmod_ref.at[:, pl.ds(MOD1, 6 * D - MOD1)],
                 in_sems.at[6])
    cp_w = [copy(w_hbm.at[:, pl.ds(fh * FH, FH)], w_ref.at[fh], w_sems.at[k * NFH + fh])
            for fh in range(NFH)
            for k, (w_hbm, w_ref) in enumerate(((wg_hbm, wg_ref), (wu_hbm, wu_ref), (wdt_hbm, wdt_ref)))]

    cp_q.start()
    cp_c.start()
    cp_k.start()
    cp_v.start()
    cp_m1.start()

    for cidx in range(NCH - LAG, NCH):
        s_ref[cidx % RING] = jnp.zeros((KC, TQ), F32)
        for _, g in TILES[cidx]:
            sb_ref[3, g * 16:(g + 1) * 16, :] = jnp.zeros((16, TQ), F32)
    pneg_ref[...] = jnp.zeros((8, TQ), F32)
    pacc_ref[...] = jnp.ones((VR, TQ), F32)
    bad_ref[...] = jnp.zeros((8, TQ), F32)

    cp_q.wait()
    cp_x[0].start()
    cp_x[1].start()
    wqkv_ref[NKV:NQKV, :] = wq_ref[...].astype(F32).T.astype(BF16)
    cp_k.wait()
    cp_v.wait()
    zpad = jnp.zeros((KW - DH, D), F32)
    kv_t = jnp.concatenate(
        [wkv_ref[0].astype(F32), zpad, wkv_ref[1].astype(F32), zpad], axis=0)
    wqkv_ref[0:NKV, :] = kv_t.astype(BF16)

    cp_c.wait()
    sc = jnp.broadcast_to(_silu(c_ref[0].astype(F32)), (8, D))

    def mod_cols(lo, hi):
        mod = _dot(sc, wmod_ref[:, lo:hi])
        mod_ref[lo:hi, :] = jnp.broadcast_to(mod[0:1, :], (128, hi - lo)).T

    cp_m1.wait()
    for i in range(2, NM):
        cp_x[i].start()
    mod_cols(0, MOD1)

    def ln1(i):
        sa = _lanes(mod_ref[0:D, :], TM)
        ca1 = 1.0 + _lanes(mod_ref[D:2 * D, :], TM)
        h1_ref[i] = (_ln_t(xt_ref[i].astype(F32)) * ca1 + sa).astype(BF16)

    def proj(i):
        tok = slice(i * TM, (i + 1) * TM)
        h = h1_ref[i]
        kv = _dot(wqkv_ref[0:NKV, :], h)
        row = jax.lax.broadcasted_iota(jnp.int32, (VR, TM), 0)
        vt_ref[:, tok] = jnp.where(row == DH, 1.0, kv[KW:NKV, :])
        kt = jnp.concatenate(
            [kv[0:KW, :] * QK_SCALE, jnp.zeros((128 - KW, TM), F32)], axis=0)
        k = kt.T
        lane = jax.lax.broadcasted_iota(jnp.int32, (TM, 128), 1)
        packed = []
        for cidx in range(i * TM // KC, (i + 1) * TM // KC):
            for n, (kind, g) in enumerate(TILES[cidx]):
                packed.append((cidx * KC - i * TM + MSZ[cidx] + 16 * n,
                               16 * g + (0 if kind == "v" else NV)))
        for r in range(4):
            kr = k if r == 0 else pltpu.roll(k, 2 * r, 1)
            kr = jnp.where(lane == ONE[r], 1.0, kr)[:, 0:KW].astype(BF16)
            ks_ref[r, tok, :] = kr
            for src, dst in packed:
                if dst < NV or r == 0:
                    ksp_ref[r, dst:dst + 16, :] = kr[src:src + 16, :]
        for src, dst in packed:
            k0_ref[dst:dst + 16, :] = k[src:src + 16, :]
        qb, off = divmod(i * TM, TQ)
        qt_ref[qb, :, off:off + TM] = _dot(wqkv_ref[NKV:NQKV, :], h)

    def q_window(t4, r, lanes=slice(None)):
        base = _aligned((t4 % (H // 4)) * (4 * DH) + 16 * r, 8)
        return qt_ref[t4 // (H // 4), pl.ds(base, KW), lanes]

    wrow = jax.lax.broadcasted_iota(jnp.int32, (KW, TQ), 0)

    def sv_mxu(g4):
        for r in range(4):
            s = _dot(ksp_ref[r, 0:NV, :], jnp.where(wrow == ONE[r], 0.0, q_window(g4, r)))
            sv_ref[4 * g4 + r] = s
            mv_ref[4 * g4 + r] = _rowmax8(s[0:8 * NMX, :])

    cp_x[0].wait()
    ln1(0)
    cp_x[1].wait()
    ln1(1)
    proj(0)
    for i in range(2, NM):
        cp_x[i].wait()
    cp_o.start()
    cp_m2.start()
    for i in range(1, NM - 1):
        ln1(i + 1)
        proj(i)
    cp_o.wait()
    cp_m2.wait()
    for cp in cp_w:
        cp.start()
    proj(NM - 1)
    mod_cols(MOD1, 6 * D)
    wot_ref[...] = wo_ref[...].astype(F32).T.astype(BF16)
    for g4 in range(H // 4):
        sv_mxu(g4)
    sb_ref[0] = _dot(ksp_ref[0, NV:NV + NC, :], jnp.where(wrow == ONE[0], 0.0, q_window(0, 0)))
    for d in range(DH):
        kb_ref[d] = jnp.broadcast_to(k0_ref[:, d:d + 1], (NV + NC, 128))

    def pv_tile(hs, cidx):
        parts = [s_ref[cidx % RING, 0:MSZ[cidx], :]]
        neg16 = jnp.concatenate([hs["neg"], hs["neg"]], axis=0)
        for kind, g in TILES[cidx]:
            rows = slice(g * 16, (g + 1) * 16)
            raw = sv_ref[hs["head"], rows, :] if kind == "v" else sb_ref[hs["u"] % 4, rows, :]
            parts.append(raw + neg16)
        p = jnp.exp2(jnp.concatenate(parts, axis=0)).astype(BF16)
        o = _dot(vt_ref[:, cidx * KC:(cidx + 1) * KC], p)
        hs["acc"] = o if hs["acc"] is None else hs["acc"] + o

    def store_o(g4, r, acc):
        ot_ref[g4, r * DH:(r + 1) * DH, :] = acc[0:DH, :] * (1.0 / acc[DH:DH + 1, :])

    def flag(acc, bad):
        l = acc[16:24, :]
        ok = jnp.logical_and(l >= L_LO, l <= L_HI)
        row8 = jax.lax.broadcasted_iota(jnp.int32, (8, TQ), 0)
        return jnp.where(jnp.logical_or(ok, row8 != DH - 16), bad, 1.0)

    def attn_block(it):
        zero = jax.lax.shift_right_logical(it, 16)
        t4 = it * (HPI // 4)
        h0 = (it % IPB) * HPI
        bad = bad_ref[...]
        hs = {"acc": pacc_ref[...], "u": -1, "head": None, "neg": pneg_ref[...]}
        pend = [(hs, cidx) for cidx in range(NCH - LAG, NCH)]
        for u in range(HPI):
            r = u % 4
            mx = jnp.max(mv_ref[h0 + u], axis=0, keepdims=True)
            neg = jnp.broadcast_to(-mx, (8, TQ))
            neg = pltpu.bitcast(pltpu.bitcast(neg, jnp.int32) & jnp.int32(-65536), F32)
            q = jnp.where(wrow == ONE[r], jnp.concatenate([neg] * (KW // 8), axis=0),
                          q_window(t4 + u // 4, r))
            hs = {"acc": None, "u": u, "head": h0 + u, "neg": neg}
            rn = (u + 1) % 4
            tn4 = t4 + (u + 1) // 4
            if u == HPI - 1:
                tn4 = jnp.minimum(tn4, NT // 4 - 1)
            for cidx in range(NCH):
                s = _dot(ks_ref[r, cidx * KC:cidx * KC + MSZ[cidx], :], q)
                s_ref[cidx % RING, 0:MSZ[cidx], :] = s
                for pi, (j, kb) in enumerate(PIECES):
                    if not MG0[cidx] <= PIECE_POS[pi] < MG0[cidx] + MSZ[cidx] // 8:
                        continue
                    if kb == 0:
                        qw = q_window(tn4, rn, slice(j * 128, (j + 1) * 128))
                        qd = jnp.stack([
                            jnp.broadcast_to(qw[2 * rn + d:2 * rn + d + 1, :], (8, 128))
                            for d in range(DH)])
                    sv = jnp.sum(kb_ref[:, NV + kb * 8:NV + (kb + 1) * 8, :] * qd, axis=0)
                    ar = (PIECE_POS[pi] - MG0[cidx]) * 8
                    sv = sv + _tie(s[ar:ar + 8, (pi % NTL) * 128:(pi % NTL + 1) * 128], zero)
                    sb_ref[rn, kb * 8:(kb + 1) * 8, j * 128:(j + 1) * 128] = sv
                pend.append((hs, cidx))
                hp, cp = pend.pop(0)
                pv_tile(hp, cp)
                if cp == NCH - 1:
                    g4 = t4 + hp["u"] // 4
                    if hp["u"] < 0:
                        g4 = jnp.maximum(g4, 0)
                    store_o(g4, hp["u"] % 4, hp["acc"])
                    bad = flag(hp["acc"], bad)
        pacc_ref[...] = hs["acc"]
        pneg_ref[...] = hs["neg"]
        bad_ref[...] = bad

    def attn_exact(qb):
        def head(h, carry):
            r = h % 4
            base = pl.multiple_of((h // 4) * (4 * DH) + 16 * r, 8)
            one = jnp.where(r == 3, ONE[3], ONE[0])
            q = jnp.where(wrow == one, 0.0, qt_ref[qb, pl.ds(base, KW), :])

            def scores(cidx):
                return _dot(ks_ref[r, pl.ds(pl.multiple_of(cidx * KC, KC), KC), :], q)

            m = jax.lax.fori_loop(
                0, NCH, lambda cidx, m: jnp.maximum(m, _rowmax8(scores(cidx))),
                jnp.full((8, TQ), -jnp.inf, F32))
            m = jnp.max(m, axis=0, keepdims=True)

            def pv(cidx, acc):
                p = jnp.exp2(scores(cidx) - m).astype(BF16)
                return acc + _dot(vt_ref[:, pl.ds(pl.multiple_of(cidx * KC, KC), KC)], p)

            acc = jax.lax.fori_loop(0, NCH, pv, jnp.zeros((VR, TQ), F32))
            for rr in range(4):
                @pl.when(r == rr)
                def _():
                    store_o(qb * (H // 4) + h // 4, rr, acc)
            return carry

        jax.lax.fori_loop(0, H, head, 0)

    def c1(qb, half):
        mb = 2 * qb + half
        ga = _lanes(mod_ref[2 * D:3 * D, :], TM)
        o = ot_ref[pl.ds(qb * (H // 4), H // 4), :, half * TM:(half + 1) * TM].reshape(D, TM)
        x1 = xt_ref[mb].astype(F32) + ga * _dot(wot_ref[...], o)
        for e in range(NFH):
            x1_ref[NFH * mb + e] = x1[:, e * 128:(e + 1) * 128]

    def c2(src, dst):
        sb = mod_ref[3 * D:4 * D, :]
        cb1 = 1.0 + mod_ref[4 * D:5 * D, :]
        h2_ref[dst] = (_ln_t(x1_ref[src]) * cb1 + sb).T.astype(BF16)

    def finish_block(qb):
        hs = {"acc": pacc_ref[...], "u": -1, "head": None, "neg": pneg_ref[...]}
        for cidx in range(NCH - LAG, NCH):
            pv_tile(hs, cidx)
        store_o(qb * (H // 4) + H // 4 - 1, 3, hs["acc"])
        bad = jnp.max(flag(hs["acc"], bad_ref[...]))
        bad_ref[...] = jnp.zeros((8, TQ), F32)

        @pl.when(bad > 0.0)
        def _():
            attn_exact(qb)

        c1(qb, 0)
        c1(qb, 1)
        for e in range(DPB):
            c2(DPB * qb + e, DPB * qb + e)

    def out_copy(mb):
        return copy(stage_ref.at[mb], out_hbm.at[0, :, pl.ds(_aligned(mb * TM, TM), TM)],
                    out_sems.at[mb])

    def vpu_scores(i, segs):
        zero = jax.lax.shift_right_logical(i, 16)
        qb_next = jnp.minimum(i // DPB + 1, NQB - 1)
        t4base = qb_next * (H // 4) + (i % DPB) * (H // 4 // DPB)
        pieces = [(hh, j, kb) for hh in range(H // DPB) for j in range(NTL) for kb in range(NV // 8)]
        total = sum(w for _, w in segs)
        si, cum = 0, 0.0
        for pi, (hh, j, kb) in enumerate(pieces):
            tgt = (pi + 0.5) * total / len(pieces)
            while cum + segs[si][1] < tgt:
                cum += segs[si][1]
                si += 1
            val = segs[si][0]
            ar = int((tgt - cum) / segs[si][1] * (val.shape[0] // 8)) * 8
            ln = (pi % (val.shape[1] // 128)) * 128
            t4, r = t4base + hh // 4, hh % 4
            head = (t4 % (H // 4)) * 4 + r
            lanes = slice(j * 128, (j + 1) * 128)
            if kb == 0:
                qw = q_window(t4, r, lanes)
                qd = jnp.stack([
                    jnp.broadcast_to(qw[2 * r + d:2 * r + d + 1, :], (8, 128)) for d in range(DH)])
            sv = jnp.sum(kb_ref[:, kb * 8:(kb + 1) * 8, :] * qd, axis=0)
            sv = sv + _tie(val[ar:ar + 8, ln:ln + 128], zero)
            sv_ref[head, kb * 8:(kb + 1) * 8, lanes] = sv
            if kb < NMX:
                m = sv if kb == 0 else jnp.maximum(m, sv)
            if kb == NMX - 1:
                mv_ref[head, :, lanes] = m

    def ffn(i, carry):
        mb = i // NFH
        fh = i % NFH
        h = h2_ref[pl.ds(NFH * mb, NFH)].reshape(TM, D)
        hm, ht = h[:, 0:512], h[:, 512:D]
        segs = []
        acc = None
        ready = None
        pend = []

        def down(cols, a):
            if a.shape[1] == FU:
                y = _dot_nt(wdt_ref[fh, :, cols], a)
                segs.append((y, float(D)))
                return y
            ys = [_dot_nt(wdt_ref[fh, :, cols], a[n * 128:(n + 1) * 128, :]) for n in range(2)]
            segs.extend((y, float(D)) for y in ys)
            return jnp.concatenate(ys, axis=1)

        nu = FH // FU
        for un in range(nu):
            c0 = un * FU
            wt = jnp.concatenate(
                [wg_ref[fh, 512:D, c0:c0 + FU], wu_ref[fh, 512:D, c0:c0 + FU]], axis=1)
            t = _dot(ht, wt)
            segs.append((t, float(TM)))
            parts = []
            for n in range(2):
                cols = slice(c0 + n * 128, c0 + (n + 1) * 128)
                g = _dot(hm, wg_ref[fh, 0:512, cols])
                u = _dot(hm, wu_ref[fh, 0:512, cols])
                segs.extend([(g, float(TM)), (u, WS * TM)])
                g = g + t[:, n * 128:(n + 1) * 128]
                u = u + t[:, FU + n * 128:FU + (n + 1) * 128]
                parts.append(_silu(g) * u)
                if ready is not None and n == (1 if un == nu - 1 else 0):
                    y = down(*ready)
                    acc = y if acc is None else acc + y
                    ready = None
            pend.extend(parts)
            if len(pend) == 4 or un == nu - 1:
                a = jnp.concatenate(pend, axis=1).astype(BF16)
                ready = (slice(c0 + FU - a.shape[1], c0 + FU), a)
                pend = []
        acc = acc + down(*ready)
        vpu_scores(i, segs)
        gb = mod_ref[5 * D:6 * D, :]
        for e in range(NFH):
            x2 = x1_ref[NFH * mb + e] + gb * acc[:, e * 128:(e + 1) * 128]
            x1_ref[NFH * mb + e] = x2
            stage_ref[mb, :, e * 128:(e + 1) * 128] = x2.astype(BF16)

        @pl.when(fh == NFH - 1)
        def _():
            out_copy(mb).start()

        return carry

    def main_loop(it, carry):
        attn_block(it)

        @pl.when(it % IPB == IPB - 1)
        def _():
            @pl.when(it == IPB - 1)
            def _():
                for cp in cp_w:
                    cp.wait()

            qb = it // IPB
            finish_block(qb)
            jax.lax.fori_loop(qb * DPB, (qb + 1) * DPB, ffn, 0)

        return carry

    jax.lax.fori_loop(0, NT // HPI, main_loop, 0)
    for mb in range(NM):
        out_copy(mb).wait()


@jax.jit
def pallas_adaLN_cond__grouped_kv_mqa__swiglu_ffn__prompt_kernel(
    A_x: jax.Array,
    A_wq: jax.Array,
    A_wk: jax.Array,
    A_wv: jax.Array,
    A_wo: jax.Array,
    B_x: jax.Array,
    B_w_gate: jax.Array,
    B_w_up: jax.Array,
    B_w_down: jax.Array,
    c: jax.Array,
    w_mod: jax.Array,
):
    del B_x
    hbm = pl.BlockSpec(memory_space=pltpu.HBM)
    out_t = pl.pallas_call(
        _kernel,
        out_shape=jax.ShapeDtypeStruct((1, D, S), A_x.dtype),
        in_specs=[hbm] * 10,
        out_specs=hbm,
        scratch_shapes=[
            pltpu.VMEM((NM, D, TM), BF16),
            pltpu.VMEM((D, D), BF16),
            pltpu.VMEM((8, DH, D), BF16),
            pltpu.VMEM((D, D), BF16),
            pltpu.VMEM((NFH, D, FH), BF16),
            pltpu.VMEM((NFH, D, FH), BF16),
            pltpu.VMEM((NFH, D, FH), BF16),
            pltpu.VMEM((32, 1, D), BF16),
            pltpu.VMEM((D, 6 * D), BF16),
            pltpu.SemaphoreType.DMA((7,)),
            pltpu.SemaphoreType.DMA((NM,)),
            pltpu.SemaphoreType.DMA((3 * NFH,)),
            pltpu.SemaphoreType.DMA((NM,)),
            pltpu.VMEM((6 * D, 128), F32),
            pltpu.VMEM((640, D), BF16),
            pltpu.VMEM((D, D), BF16),
            pltpu.VMEM((NM, D, TM), BF16),
            pltpu.VMEM((4, S, KW), BF16),
            pltpu.VMEM((4, NV + NC, KW), BF16),
            pltpu.VMEM((NV + NC, 128), F32),
            pltpu.VMEM((DH, NV + NC, 128), F32),
            pltpu.VMEM((VR, S), F32),
            pltpu.VMEM((NQB, D, TQ), F32),
            pltpu.VMEM((RING, KC, TQ), F32),
            pltpu.VMEM((H, NV, TQ), F32),
            pltpu.VMEM((H, 8, TQ), F32),
            pltpu.VMEM((4, NC, TQ), F32),
            pltpu.VMEM((VR, TQ), F32),
            pltpu.VMEM((8, TQ), F32),
            pltpu.VMEM((8, TQ), F32),
            pltpu.VMEM((NT // 4, 4 * DH, TQ), F32),
            pltpu.VMEM((NFH * NM, D, 128), F32),
            pltpu.VMEM((NFH * NM, 128, D), BF16),
            pltpu.VMEM((NM, D, TM), BF16),
        ],
        compiler_params=pltpu.CompilerParams(
            vmem_limit_bytes=100 * 1024 * 1024, internal_scratch_in_bytes=65536),
    )(
        jnp.transpose(A_x, (0, 2, 1)), A_wq, A_wk.T, A_wv.T, A_wo,
        B_w_gate, B_w_up, B_w_down.T, c, w_mod,
    )
    return jnp.transpose(out_t, (0, 2, 1))
```

```python
import math

import jax
import jax.numpy as jnp
import jax.experimental.pallas as pl
import jax.experimental.pallas.tpu as pltpu

F32 = jnp.float32
BF16 = jnp.bfloat16

S = 2048
D = 576
H = 32
DH = D // H
FF = 4608
EPS = 1e-05

KW = 24
VR = 24
NKV = 2 * KW
NQKV = NKV + D
ONE = (23, 23, 23, 0)

TM = 256
NM = S // TM
TQ = 512
NQB = S // TQ
NTL = TQ // 128
SPB = H * TM // TQ
KC = 128
NCH = S // KC
HPI = 8
IPB = SPB // HPI
LAG = 3
RING = 8
NT = NM * SPB
FU = 256
WS = 0.8
NFH = 2
FH = FF // NFH
MOD0 = 768
MOD1 = 2 * D

NV = 320
NVF = 32
NF0 = 4
NMX = 8
NC = 192


def _tile_groups():
    gv, gc = NV // 16, NC // 16
    per = [((c + 1) * (gv + gc)) // NCH - (c * (gv + gc)) // NCH for c in range(NCH)]
    tail = sum(per[NCH - LAG:])
    kinds, a, b = [], 0, 0
    for _ in range(gv + gc - tail):
        if a < gv and (a * (gc - tail) <= b * gv or b >= gc - tail):
            kinds.append("v")
            a += 1
        else:
            kinds.append("c")
            b += 1
    kinds += ["c"] * tail
    tiles, i, idx = [], 0, {"v": 0, "c": 0}
    for c in range(NCH):
        tiles.append([])
        for _ in range(per[c]):
            tiles[c].append((kinds[i], idx[kinds[i]]))
            idx[kinds[i]] += 1
            i += 1
    assert idx == {"v": gv, "c": gc}
    return tiles


TILES = _tile_groups()
MSZ = [KC - 16 * len(t) for t in TILES]
MG0 = [sum(MSZ[:c]) // 8 for c in range(NCH)]
PIECES = [(j, kb) for j in range(NTL) for kb in range(NC // 8)]
PIECE_POS = [((pi + 1) * (sum(MSZ) // 8)) // len(PIECES) - 1 for pi in range(len(PIECES))]

QK_SCALE = (DH ** -0.5) * math.log2(math.e)
L_LO, L_HI = 2.0 ** -64, 2.0 ** 64


def _dot(a, b):
    return jnp.dot(a, b, preferred_element_type=F32)


def _dot_nt(a, b):
    return jax.lax.dot_general(a, b, (((1,), (1,)), ((), ())), preferred_element_type=F32)


def _stats(x):
    pivot = x[0:1, :]
    d = x - pivot
    m = jnp.mean(d, axis=0, keepdims=True)
    v = jnp.maximum(jnp.mean(d * d, axis=0, keepdims=True) - m * m, 0.0)
    return pivot + m, jax.lax.rsqrt(v + EPS)


def _silu(g):
    h = 0.5 * g
    return h + h * jnp.tanh(h)


def _normalize(acc):
    l = acc[DH:DH + 1, :]
    r = pl.reciprocal(l, approx=True)
    r = r * (2.0 - l * r)
    return acc[0:DH, :] * r


def _pack_store(ref, row0, w):
    w = jnp.concatenate([w, jnp.zeros((w.shape[0], 640 - D), F32)], axis=1).astype(BF16)
    for k in range(5):
        ref[k, row0 // 2:(row0 + w.shape[0]) // 2, :] = pltpu.bitcast(
            w[:, k * 128:(k + 1) * 128], jnp.int32)


def _pack_load(ref, r0, r1, c0, c1):
    w = [pltpu.bitcast(ref[k, r0 // 2:r1 // 2, :], BF16) for k in range(c0 // 128, -(-c1 // 128))]
    return jnp.concatenate(w, axis=1)[:, 0:c1 - c0]


def _rowmax8(s):
    return jnp.max(s.reshape(s.shape[0] // 8, 8, s.shape[1]), axis=0)


def _aligned(x, n):
    return x if isinstance(x, int) else pl.multiple_of(x, n)


def _tie(x, zero):
    return pltpu.bitcast(pltpu.bitcast(x, jnp.int32) & zero, F32)


def _kernel(
    xt_hbm, wq_hbm, wkt_hbm, wvt_hbm, wo_hbm, wg_hbm, wu_hbm, wdt_hbm, c_hbm, wmod_hbm,
    out_hbm,
    xt_ref, wq_ref, wkv_ref, wo_ref, wg_ref, wu_ref, wdt_ref, c_ref, wmod_ref,
    in_sems, x_sems, w_sems, out_sems,
    mod_ref, wqkv_ref, wot_ref, h1_ref, ks_ref, ksp_ref, k0_ref, kb_ref, vt_ref, qt_ref,
    s_ref, sv_ref, mv_ref, sb_ref, pacc_ref, pneg_ref, bad_ref, ot_ref,
    x1_ref, st_ref, h2_ref, stage_ref,
):
    def copy(src, dst, sem):
        return pltpu.make_async_copy(src, dst, sem)

    cp_c = copy(c_hbm, c_ref.at[0], in_sems.at[0])
    cp_m0 = copy(wmod_hbm.at[:, pl.ds(0, MOD0)], wmod_ref.at[:, pl.ds(0, MOD0)], in_sems.at[7])
    cp_m1 = copy(wmod_hbm.at[:, pl.ds(MOD0, MOD1 - MOD0)], wmod_ref.at[:, pl.ds(MOD0, MOD1 - MOD0)],
                 in_sems.at[1])
    cp_q = copy(wq_hbm, wq_ref, in_sems.at[2])
    cp_k = copy(wkt_hbm, wkv_ref.at[0], in_sems.at[3])
    cp_v = copy(wvt_hbm, wkv_ref.at[1], in_sems.at[4])
    cp_x = [copy(xt_hbm.at[0, :, pl.ds(i * TM, TM)], xt_ref.at[i], x_sems.at[i]) for i in range(NM)]
    cp_o = copy(wo_hbm, wo_ref, in_sems.at[5])
    cp_m2 = copy(wmod_hbm.at[:, pl.ds(MOD1, 6 * D - MOD1)], wmod_ref.at[:, pl.ds(MOD1, 6 * D - MOD1)],
                 in_sems.at[6])
    cp_w = [copy(w_hbm.at[:, pl.ds(fh * FH, FH)], w_ref.at[fh], w_sems.at[k * NFH + fh])
            for fh in range(NFH)
            for k, (w_hbm, w_ref) in enumerate(((wg_hbm, wg_ref), (wu_hbm, wu_ref), (wdt_hbm, wdt_ref)))]

    for cp in [cp_q, cp_c, cp_k, cp_v, cp_m0]:
        cp.start()

    for cidx in range(NCH - LAG, NCH):
        s_ref[cidx % RING] = jnp.zeros((KC, TQ), F32)
        for _, g in TILES[cidx]:
            sb_ref[3, g * 16:(g + 1) * 16, :] = jnp.zeros((16, TQ), F32)
    pneg_ref[...] = jnp.zeros((8, TQ), F32)
    pacc_ref[...] = jnp.ones((VR, TQ), F32)
    bad_ref[...] = jnp.zeros((8, TQ), F32)
    for mb in range(NM):
        ot_ref[(mb + 1) * (SPB // 4) - 1, 48:4 * DH, :] = jnp.zeros((4 * DH - 48, TQ), F32)

    def stats1(e):
        x = xt_ref[e // 2, :, (e % 2) * 128:(e % 2 + 1) * 128].astype(F32)
        mean, rstd = _stats(x)
        st_ref[e, 0:1, :] = mean
        st_ref[e, 8:9, :] = rstd
        return rstd

    cp_k.wait()
    cp_v.wait()
    cp_c.wait()
    zpad = jnp.zeros((KW - DH, D), F32)
    kv_t = jnp.concatenate(
        [wkv_ref[0].astype(F32), zpad, wkv_ref[1].astype(F32), zpad], axis=0)
    _pack_store(wqkv_ref, 0, kv_t)
    sc = jnp.broadcast_to(_silu(c_ref[0].astype(F32)), (8, D))
    cp_q.wait()
    cp_x[0].start()
    cp_m1.start()
    _pack_store(wqkv_ref, NKV, wq_ref[...].astype(F32).T)

    def mod_cols(lo, hi):
        mod = _dot(sc, wmod_ref[:, lo:hi])
        col = lo + jax.lax.broadcasted_iota(jnp.int32, (8, hi - lo), 1)
        scale = jnp.logical_or(jnp.logical_and(col >= D, col < 2 * D),
                               jnp.logical_and(col >= 4 * D, col < 5 * D))
        mod = jnp.where(scale, 1.0 + mod, mod)
        mod_ref[lo:hi, :] = jnp.broadcast_to(mod[0:1, :], (128, hi - lo)).T

    cp_m0.wait()
    cp_x[1].start()
    mod_cols(0, MOD0)
    cp_x[0].wait()
    cp_x[2].start()
    cp_x[3].start()
    stats1(0)
    stats1(1)
    cp_m1.wait()
    for cp in cp_x[4:]:
        cp.start()
    mod_cols(MOD0, MOD1)

    def ln1(e, z=None):
        x = xt_ref[e // 2, :, (e % 2) * 128:(e % 2 + 1) * 128].astype(F32)
        mean = st_ref[e, 0:1, :] if z is None else st_ref[e, 0:1, :] + z
        h = ((x - mean) * (st_ref[e, 8:9, :] * mod_ref[D:2 * D, :])
             + mod_ref[0:D, :])
        h1_ref[e] = pltpu.bitcast(h.astype(BF16), jnp.int32)

    def proj_main(e):
        return _dot(_pack_load(wqkv_ref, 0, NQKV, 0, 512), pltpu.bitcast(h1_ref[e, 0:256, :], BF16))

    def proj_tail(qb):
        return _dot(_pack_load(wqkv_ref, 0, NQKV, 512, D), _pack_load(h1_ref, 512, D, qb * TQ, (qb + 1) * TQ))

    def proj_out(e, qkv):
        tok = slice(e * KC, (e + 1) * KC)
        row = jax.lax.broadcasted_iota(jnp.int32, (VR, 128), 0)
        vt_ref[:, tok] = jnp.where(row == DH, 1.0, qkv[KW:NKV, :])
        kt = jnp.concatenate(
            [qkv[0:KW, :] * QK_SCALE, jnp.zeros((128 - KW, 128), F32)], axis=0)
        k = kt.T
        lane = jax.lax.broadcasted_iota(jnp.int32, (128, 128), 1)
        packed = [(MSZ[e] + 16 * n, 16 * g + (0 if kind == "v" else NV))
                  for n, (kind, g) in enumerate(TILES[e])]
        for r in range(4):
            kr = k if r == 0 else pltpu.roll(k, 2 * r, 1)
            kr = jnp.where(lane == ONE[r], 1.0, kr).astype(BF16)
            ks_ref[r, e * (KC // 2):(e + 1) * (KC // 2), :] = pltpu.bitcast(kr, jnp.int32)
            for src, dst in packed:
                if dst < NV or r == 0:
                    ksp_ref[r, dst:dst + 16, :] = kr[src:src + 16, :]
        for src, dst in packed:
            k0_ref[dst:dst + 16, :] = k[src:src + 16, :]
        for g in range(H // 4):
            lo = (g % 2) * TM + (e % 2) * 128
            qt_ref[(e // 2) * (SPB // 4) + g // 2, :, lo:lo + 128] = (
                qkv[NKV + g * 4 * DH:NKV + (g + 1) * 4 * DH, :])

    def q_window(t4, r, lanes=slice(None)):
        return qt_ref[t4, 16 * r:16 * r + KW, lanes]

    wrow = jax.lax.broadcasted_iota(jnp.int32, (KW, TQ), 0)

    def sv_mxu(g4):
        for r in range(4):
            s = _dot(ksp_ref[r, 0:NV, 0:KW], jnp.where(wrow == ONE[r], 0.0, q_window(g4, r)))
            sv_ref[4 * g4 + r] = s
            mv_ref[4 * g4 + r] = _rowmax8(s[0:8 * NMX, :])

    zero_a = (c_ref[0, :, 0:128].astype(F32) > 3e38).astype(jnp.int32) >> 1
    ln1(0)
    a = [proj_main(0)]
    ln1(1)
    cp_x[1].wait()
    a.append(proj_main(1))
    stats1(2)
    stats1(3)
    ln1(2)
    ln1(3, _tie(a[1][64:65, :], zero_a))
    tail = proj_tail(0)
    for e in range(2):
        proj_out(e, a[e] + tail[:, e * 128:(e + 1) * 128])
    cp_x[2].wait()
    cp_x[3].wait()
    for e in range(2, NCH):
        if e == 4:
            for cp in cp_x[4:]:
                cp.wait()
            cp_o.start()
            cp_m2.start()
        if e % 4 == 0:
            for n in range(e, e + 4):
                ln1(n)
            tail = proj_tail(e // 4)
        qkv = proj_main(e) + tail[:, (e % 4) * 128:(e % 4 + 1) * 128]
        nxt = {2: (4, 5), 3: (6, 7)}.get(e, (e + 4,) if e + 4 < NCH else ())
        for n, row in zip(nxt, (600, 320)):
            z = _tie(stats1(n), zero_a)
            qkv = jnp.concatenate([qkv[0:row, :], qkv[row:row + 8, :] + z, qkv[row + 8:, :]], axis=0)
        proj_out(e, qkv)
    cp_o.wait()
    cp_m2.wait()
    for cp in cp_w:
        cp.start()
    sv_mxu(0)
    mod_cols(MOD1, 6 * D)
    _pack_store(wot_ref, 0, wo_ref[...].astype(F32).T)
    for g4 in range(1, SPB // 4):
        sv_mxu(g4)
    sb_ref[0] = _dot(ksp_ref[0, NV:NV + NC, 0:KW], jnp.where(wrow == ONE[0], 0.0, q_window(0, 0)))
    for d in range(DH):
        kb_ref[d] = jnp.broadcast_to(k0_ref[:, d:d + 1], (NV + NC, 128))

    def pv_tile(hs, cidx):
        parts = [s_ref[cidx % RING, 0:MSZ[cidx], :]]
        neg16 = jnp.concatenate([hs["neg"], hs["neg"]], axis=0)
        for kind, g in TILES[cidx]:
            rows = slice(g * 16, (g + 1) * 16)
            raw = sv_ref[hs["head"], rows, :] if kind == "v" else sb_ref[hs["u"] % 4, rows, :]
            parts.append(raw + neg16)
        p = jnp.exp2(jnp.concatenate(parts, axis=0)).astype(BF16)
        o = _dot(vt_ref[:, cidx * KC:(cidx + 1) * KC], p)
        hs["acc"] = o if hs["acc"] is None else hs["acc"] + o

    def store_o(g4, r, acc):
        ot_ref[g4, r * DH:(r + 1) * DH, :] = _normalize(acc)

    def flag(acc, bad):
        l = acc[16:24, :]
        ok = jnp.logical_and(l >= L_LO, l <= L_HI)
        row8 = jax.lax.broadcasted_iota(jnp.int32, (8, TQ), 0)
        return jnp.where(jnp.logical_or(ok, row8 != DH - 16), bad, 1.0)

    def attn_block(it):
        zero = jax.lax.shift_right_logical(it, 16)
        t4 = it * (HPI // 4)
        h0 = (it % IPB) * HPI
        bad = bad_ref[...]
        hs = {"acc": pacc_ref[...], "u": -1, "head": None, "neg": pneg_ref[...]}
        pend = [(hs, cidx) for cidx in range(NCH - LAG, NCH)]
        for u in range(HPI):
            r = u % 4
            mx = jnp.max(mv_ref[h0 + u], axis=0, keepdims=True)
            neg = jnp.broadcast_to(-mx, (8, TQ))
            neg = pltpu.bitcast(pltpu.bitcast(neg, jnp.int32) & jnp.int32(-65536), F32)
            q = jnp.where(wrow == ONE[r], jnp.concatenate([neg] * (KW // 8), axis=0),
                          q_window(t4 + u // 4, r))
            hs = {"acc": None, "u": u, "head": h0 + u, "neg": neg}
            rn = (u + 1) % 4
            tn4 = t4 + (u + 1) // 4
            if u == HPI - 1:
                tn4 = jnp.minimum(tn4, NT // 4 - 1)
            for cidx in range(NCH):
                kk = ks_ref[r, cidx * (KC // 2):cidx * (KC // 2) + MSZ[cidx] // 2, :]
                s = _dot(pltpu.bitcast(kk, BF16)[:, 0:KW], q)
                s_ref[cidx % RING, 0:MSZ[cidx], :] = s
                for pi, (j, kb) in enumerate(PIECES):
                    if not MG0[cidx] <= PIECE_POS[pi] < MG0[cidx] + MSZ[cidx] // 8:
                        continue
                    if kb == 0:
                        qw = q_window(tn4, rn, slice(j * 128, (j + 1) * 128))
                        qd = jnp.stack([
                            jnp.broadcast_to(qw[2 * rn + d:2 * rn + d + 1, :], (8, 128))
                            for d in range(DH)])
                    sv = jnp.sum(kb_ref[:, NV + kb * 8:NV + (kb + 1) * 8, :] * qd, axis=0)
                    ar = (PIECE_POS[pi] - MG0[cidx]) * 8
                    sv = sv + _tie(s[ar:ar + 8, (pi % NTL) * 128:(pi % NTL + 1) * 128], zero)
                    sb_ref[rn, kb * 8:(kb + 1) * 8, j * 128:(j + 1) * 128] = sv
                pend.append((hs, cidx))
                hp, cp = pend.pop(0)
                pv_tile(hp, cp)
                if cp == NCH - 1:
                    g4 = t4 + hp["u"] // 4
                    if hp["u"] < 0:
                        g4 = jnp.maximum(g4, 0)
                    store_o(g4, hp["u"] % 4, hp["acc"])
                    bad = flag(hp["acc"], bad)
        pacc_ref[...] = hs["acc"]
        pneg_ref[...] = hs["neg"]
        bad_ref[...] = bad

    def attn_exact(mb):
        def head(h, carry):
            r = h % 4
            t4 = mb * (SPB // 4) + h // 4
            one = jnp.where(r == 3, ONE[3], ONE[0])
            q = jnp.where(wrow == one, 0.0, qt_ref[t4, pl.ds(pl.multiple_of(16 * r, 8), KW), :])

            def scores(cidx):
                kk = ks_ref[r, pl.ds(pl.multiple_of(cidx * (KC // 2), KC // 2), KC // 2), :]
                return _dot(pltpu.bitcast(kk, BF16)[:, 0:KW], q)

            m = jax.lax.fori_loop(
                0, NCH, lambda cidx, m: jnp.maximum(m, _rowmax8(scores(cidx))),
                jnp.full((8, TQ), -jnp.inf, F32))
            m = jnp.max(m, axis=0, keepdims=True)

            def pv(cidx, acc):
                p = jnp.exp2(scores(cidx) - m).astype(BF16)
                return acc + _dot(vt_ref[:, pl.ds(pl.multiple_of(cidx * KC, KC), KC)], p)

            acc = jax.lax.fori_loop(0, NCH, pv, jnp.zeros((VR, TQ), F32))
            for rr in range(4):
                @pl.when(r == rr)
                def _():
                    store_o(t4, rr, acc)
            return carry

        jax.lax.fori_loop(0, SPB, head, 0)

    def finish_block(mb):
        g0 = mb * (SPB // 4)

        def attempt(state):
            k, _ = state

            @pl.when(k == 1)
            def _():
                attn_exact(mb)

            def o_rows(lo, hi):
                o = [ot_ref[g0 + g // 2, :, (g % 2) * TM:(g % 2 + 1) * TM]
                     for g in range(lo // (4 * DH), -(-hi // (4 * DH)))]
                off = lo // (4 * DH) * (4 * DH)
                return jnp.concatenate(o, axis=0)[lo - off:hi - off, :]

            zero = jax.lax.shift_right_logical(k, 16)

            def after(x, dep):
                z = jnp.concatenate([_tie(dep, zero)] * (x.shape[1] // 128), axis=1)
                return jnp.concatenate([x[0:-8, :], x[-8:, :] + z], axis=0)

            def resid(e, attn):
                x = xt_ref[mb, :, e * 128:(e + 1) * 128].astype(F32)
                x1 = x + mod_ref[2 * D:3 * D, :] * attn
                x1_ref[e] = x1
                return _stats(x1)

            def ln2(e, mean, rstd):
                x1 = x1_ref[e + zero]
                h2 = (x1 - mean) * (rstd * mod_ref[4 * D:5 * D, :]) + mod_ref[3 * D:4 * D, :]
                _pack_store(h2_ref, e * 128, h2.T)

            tn = jnp.minimum(mb + 1, NM - 1) * (SPB // 4)

            def fill(steps):
                for h in steps:
                    q = jnp.where(wrow == ONE[h % 4], 0.0, q_window(tn + h // 4, h % 4))
                    sv_ref[h, NV - NVF:NV, :] = _dot(ksp_ref[h % 4, NV - NVF:NV, 0:KW], q)

            fill(range(NF0))
            hs = {"acc": pacc_ref[...], "u": -1, "head": None, "neg": pneg_ref[...]}
            for cidx in range(NCH - LAG, NCH):
                pv_tile(hs, cidx)
            a = _dot(_pack_load(wot_ref, 0, D, 0, 256), o_rows(0, 256))
            acc = hs["acc"]
            rows = slice(3 * DH, 4 * DH)
            gl = g0 + SPB // 4 - 1
            ot_ref[gl, rows, :] = jnp.where(
                k == 0, _normalize(acc), ot_ref[gl, rows, :])
            bad = jnp.max(flag(acc, bad_ref[...]))
            o = after(o_rows(512, D), a[256:264, 0:128])
            t = jnp.concatenate(
                [_dot(_pack_load(wot_ref, lo, lo + D // 2, 512, D), o) for lo in (0, D // 2)], axis=0)
            b = _dot(_pack_load(wot_ref, 0, D, 256, 512), after(o_rows(256, 512), t[32:40, 0:128]))
            attn = (a + t) + b
            st = [resid(e, attn[:, e * 128:(e + 1) * 128]) for e in range(TM // 128)]
            for e in range(TM // 128):
                ln2(e, *st[e])
            fill(range(NF0, SPB))
            return k + 1, (bad > 0.0).astype(jnp.int32)

        jax.lax.while_loop(lambda st: st[0] <= st[1], attempt, (jnp.int32(0), jnp.int32(0)))
        bad_ref[...] = jnp.zeros((8, TQ), F32)

    def out_copy(mb):
        return copy(stage_ref.at[mb], out_hbm.at[0, :, pl.ds(_aligned(mb * TM, TM), TM)],
                    out_sems.at[mb])

    def vpu_scores(i, segs):
        zero = jax.lax.shift_right_logical(i, 16)
        l4base = (i % NFH) * (SPB // 4 // NFH)
        t4base = jnp.minimum(i // NFH + 1, NM - 1) * (SPB // 4) + l4base
        pieces = [(hh, j, kb) for hh in range(SPB // NFH) for j in range(NTL)
                  for kb in range((NV - NVF) // 8)]
        total = sum(w for _, w in segs)
        si, cum = 0, 0.0
        for pi, (hh, j, kb) in enumerate(pieces):
            tgt = (pi + 0.5) * total / len(pieces)
            while cum + segs[si][1] < tgt:
                cum += segs[si][1]
                si += 1
            val = segs[si][0]
            ar = int((tgt - cum) / segs[si][1] * (val.shape[0] // 8)) * 8
            ln = (pi % (val.shape[1] // 128)) * 128
            t4, r = t4base + hh // 4, hh % 4
            head = 4 * l4base + hh
            lanes = slice(j * 128, (j + 1) * 128)
            if kb == 0:
                qw = q_window(t4, r, lanes)
                qd = jnp.stack([
                    jnp.broadcast_to(qw[2 * r + d:2 * r + d + 1, :], (8, 128)) for d in range(DH)])
            sv = jnp.sum(kb_ref[:, kb * 8:(kb + 1) * 8, :] * qd, axis=0)
            sv = sv + _tie(val[ar:ar + 8, ln:ln + 128], zero)
            sv_ref[head, kb * 8:(kb + 1) * 8, lanes] = sv
            if kb < NMX:
                m = sv if kb == 0 else jnp.maximum(m, sv)
            if kb == NMX - 1:
                mv_ref[head, :, lanes] = m

    def ffn(i, carry):
        mb = i // NFH
        fh = i % NFH
        hm, ht = _pack_load(h2_ref, 0, TM, 0, 512), _pack_load(h2_ref, 0, TM, 512, D)
        segs = []
        acc = None
        ready = None
        pend = []

        def down(cols, a):
            if a.shape[1] == FU:
                y = _dot_nt(wdt_ref[fh, :, cols], a)
                segs.append((y, float(D)))
                return y
            ys = [_dot_nt(wdt_ref[fh, :, cols], a[n * 128:(n + 1) * 128, :]) for n in range(2)]
            segs.extend((y, float(D)) for y in ys)
            return jnp.concatenate(ys, axis=1)

        nu = FH // FU
        for un in range(nu):
            c0 = un * FU
            wt = jnp.concatenate(
                [wg_ref[fh, 512:D, c0:c0 + FU], wu_ref[fh, 512:D, c0:c0 + FU]], axis=1)
            t = _dot(ht, wt)
            segs.append((t, float(TM)))
            parts = []
            for n in range(2):
                cols = slice(c0 + n * 128, c0 + (n + 1) * 128)
                g = _dot(hm, wg_ref[fh, 0:512, cols])
                u = _dot(hm, wu_ref[fh, 0:512, cols])
                segs.extend([(g, float(TM)), (u, WS * TM)])
                g = g + t[:, n * 128:(n + 1) * 128]
                u = u + t[:, FU + n * 128:FU + (n + 1) * 128]
                parts.append(_silu(g) * u)
                if ready is not None and n == (1 if un == nu - 1 else 0):
                    y = down(*ready)
                    acc = y if acc is None else acc + y
                    ready = None
            pend.extend(parts)
            if len(pend) == 4 or un == nu - 1:
                a = jnp.concatenate(pend, axis=1).astype(BF16)
                ready = (slice(c0 + FU - a.shape[1], c0 + FU), a)
                pend = []
        acc = acc + down(*ready)
        vpu_scores(i, segs)
        gb = mod_ref[5 * D:6 * D, :]
        for e in range(TM // 128):
            x2 = x1_ref[e] + gb * acc[:, e * 128:(e + 1) * 128]
            x1_ref[e] = x2
            stage_ref[mb, :, e * 128:(e + 1) * 128] = x2.astype(BF16)

        @pl.when(fh == NFH - 1)
        def _():
            out_copy(mb).start()

        return carry

    def main_loop(it, carry):
        attn_block(it)

        @pl.when(it % IPB == IPB - 1)
        def _():
            @pl.when(it == IPB - 1)
            def _():
                for cp in cp_w:
                    cp.wait()

            mb = it // IPB
            finish_block(mb)
            jax.lax.fori_loop(mb * NFH, (mb + 1) * NFH, ffn, 0)

        return carry

    jax.lax.fori_loop(0, NT // HPI, main_loop, 0)
    for mb in range(NM):
        out_copy(mb).wait()


@jax.jit
def pallas_adaLN_cond__grouped_kv_mqa__swiglu_ffn__prompt_kernel(
    A_x: jax.Array,
    A_wq: jax.Array,
    A_wk: jax.Array,
    A_wv: jax.Array,
    A_wo: jax.Array,
    B_x: jax.Array,
    B_w_gate: jax.Array,
    B_w_up: jax.Array,
    B_w_down: jax.Array,
    c: jax.Array,
    w_mod: jax.Array,
):
    del B_x
    hbm = pl.BlockSpec(memory_space=pltpu.HBM)
    out_t = pl.pallas_call(
        _kernel,
        out_shape=jax.ShapeDtypeStruct((1, D, S), A_x.dtype),
        in_specs=[hbm] * 10,
        out_specs=hbm,
        scratch_shapes=[
            pltpu.VMEM((NM, D, TM), BF16),
            pltpu.VMEM((D, D), BF16),
            pltpu.VMEM((8, DH, D), BF16),
            pltpu.VMEM((D, D), BF16),
            pltpu.VMEM((NFH, D, FH), BF16),
            pltpu.VMEM((NFH, D, FH), BF16),
            pltpu.VMEM((NFH, D, FH), BF16),
            pltpu.VMEM((32, 1, D), BF16),
            pltpu.VMEM((D, 6 * D), BF16),
            pltpu.SemaphoreType.DMA((8,)),
            pltpu.SemaphoreType.DMA((NM,)),
            pltpu.SemaphoreType.DMA((3 * NFH,)),
            pltpu.SemaphoreType.DMA((NM,)),
            pltpu.VMEM((6 * D, 128), F32),
            pltpu.VMEM((5, 320, 128), jnp.int32),
            pltpu.VMEM((5, D // 2, 128), jnp.int32),
            pltpu.VMEM((NCH, D // 2, 128), jnp.int32),
            pltpu.VMEM((4, S // 2, 128), jnp.int32),
            pltpu.VMEM((4, NV + NC, 128), BF16),
            pltpu.VMEM((NV + NC, 128), F32),
            pltpu.VMEM((DH, NV + NC, 128), F32),
            pltpu.VMEM((VR, S), F32),
            pltpu.VMEM((NT // 4, 4 * DH, TQ), F32),
            pltpu.VMEM((RING, KC, TQ), F32),
            pltpu.VMEM((SPB, NV, TQ), F32),
            pltpu.VMEM((SPB, 8, TQ), F32),
            pltpu.VMEM((4, NC, TQ), F32),
            pltpu.VMEM((VR, TQ), F32),
            pltpu.VMEM((8, TQ), F32),
            pltpu.VMEM((8, TQ), F32),
            pltpu.VMEM((NT // 4, 4 * DH, TQ), F32),
            pltpu.VMEM((TM // 128, D, 128), F32),
            pltpu.VMEM((16, 16, 128), F32),
            pltpu.VMEM((5, TM // 2, 128), jnp.int32),
            pltpu.VMEM((NM, D, TM), BF16),
        ],
        compiler_params=pltpu.CompilerParams(
            vmem_limit_bytes=100 * 1024 * 1024, internal_scratch_in_bytes=65536),
    )(
        jnp.transpose(A_x, (0, 2, 1)), A_wq, A_wk.T, A_wv.T, A_wo,
        B_w_gate, B_w_up, B_w_down.T, c, w_mod,
    )
    return jnp.transpose(out_t, (0, 2, 1))
```

```python
import math

import jax
import jax.numpy as jnp
import jax.experimental.pallas as pl
import jax.experimental.pallas.tpu as pltpu

F32 = jnp.float32
BF16 = jnp.bfloat16

S = 2048
D = 576
H = 32
DH = D // H
FF = 4608
EPS = 1e-05

KW = 24
VR = 24
NKV = 2 * KW
NQKV = NKV + D
ONE = (23, 23, 23, 0)

TM = 256
NM = S // TM
TQ = 512
NTL = TQ // 128
SPB = H * TM // TQ
KC = 128
NCH = S // KC
HPI = 8
IPB = SPB // HPI
LAG = 3
RING = 8
NT = NM * SPB
FU = 256
NFH = 2
FH = FF // NFH
MOD0 = 768
MOD1 = 2 * D

NV = 384
NC = 224
FV = 44
NVF = 32
NF0 = 4
V0V = 1
V0S = 6
NMX = 4
WT, WP, WB = 1.2, 1.0, 0.9


def _tile_groups():
    gv, gc = NV // 16, NC // 16
    per = [((c + 1) * (gv + gc) + 4) // NCH - (c * (gv + gc) + 4) // NCH for c in range(NCH)]
    tail = sum(per[NCH - LAG:])
    kinds, a, b = [], 0, 0
    for _ in range(gv + gc - tail):
        if a < gv and (a * (gc - tail) <= b * gv or b >= gc - tail):
            kinds.append("v")
            a += 1
        else:
            kinds.append("c")
            b += 1
    kinds += ["c"] * tail
    tiles, i, idx = [], 0, {"v": 0, "c": 0}
    for c in range(NCH):
        tiles.append([])
        for _ in range(per[c]):
            tiles[c].append((kinds[i], idx[kinds[i]]))
            idx[kinds[i]] += 1
            i += 1
    assert idx == {"v": gv, "c": gc}
    return tiles


TILES = _tile_groups()
MSZ = [KC - 16 * len(t) for t in TILES]
PIECES = [(j, kb) for j in range(NTL) for kb in range(NC // 8)]

VPIECES = [(hh, j, kb) for hh in range(SPB // NFH) for j in range(NTL)
           for kb in range((NV - NVF) // 8)]

QK_SCALE = (DH ** -0.5) * math.log2(math.e)
L_LO, L_HI = 2.0 ** -64, 2.0 ** 64


def _dot(a, b):
    return jnp.dot(a, b, preferred_element_type=F32)


def _dot_nt(a, b):
    return jax.lax.dot_general(a, b, (((1,), (1,)), ((), ())), preferred_element_type=F32)


def _stats(x):
    pivot = x[0:1, :]
    d = x - pivot
    m = jnp.mean(d, axis=0, keepdims=True)
    v = jnp.maximum(jnp.mean(d * d, axis=0, keepdims=True) - m * m, 0.0)
    return pivot + m, jax.lax.rsqrt(v + EPS)


def _silu(g):
    h = 0.5 * g
    return h + h * jnp.tanh(h)


def _normalize(acc):
    l = acc[DH:DH + 1, :]
    r = pl.reciprocal(l, approx=True)
    r = r * (2.0 - l * r)
    return acc[0:DH, :] * r


def _pack_store(ref, row0, w):
    w = jnp.concatenate([w, jnp.zeros((w.shape[0], 640 - D), F32)], axis=1).astype(BF16)
    for k in range(5):
        ref[k, row0 // 2:(row0 + w.shape[0]) // 2, :] = pltpu.bitcast(
            w[:, k * 128:(k + 1) * 128], jnp.int32)


def _pack_load(ref, r0, r1, c0, c1):
    w = [pltpu.bitcast(ref[k, r0 // 2:r1 // 2, :], BF16) for k in range(c0 // 128, -(-c1 // 128))]
    return jnp.concatenate(w, axis=1)[:, 0:c1 - c0]


def _rowmax8(s):
    return jnp.max(s.reshape(s.shape[0] // 8, 8, s.shape[1]), axis=0)


def _aligned(x, n):
    return x if isinstance(x, int) else pl.multiple_of(x, n)


def _tie(x, zero):
    return pltpu.bitcast(pltpu.bitcast(x, jnp.int32) & zero, F32)


def _always(x, zero):
    return pltpu.bitcast(x, jnp.int32) >= zero + jnp.int32(-2 ** 31)


def _pins(segs, n, ph=0.5, ls=1):
    total = sum(w for _, w in segs)
    si, cum = 0, 0.0
    for pi in range(n):
        tgt = (pi + ph) * total / n
        while cum + segs[si][1] < tgt:
            cum += segs[si][1]
            si += 1
        val = segs[si][0]
        ar = int((tgt - cum) / segs[si][1] * (val.shape[0] // 8)) * 8
        ln = (pi * ls % (val.shape[1] // 128)) * 128
        yield val[ar:ar + 8, ln:ln + 128]


def _kernel(
    xt_hbm, wq_hbm, wkt_hbm, wvt_hbm, wo_hbm, wg_hbm, wu_hbm, wdt_hbm, c_hbm, wmod_hbm,
    out_hbm,
    xt_ref, wq_ref, wkv_ref, wo_ref, wg_ref, wu_ref, wdt_ref, c_ref, wmod_ref,
    sems,
    mod_ref, wqkv_ref, wot_ref, h1_ref, ks_ref, ksp_ref, k0_ref, kb_ref, vt_ref, qt_ref,
    s_ref, sv_ref, mv_ref, sb_ref, pacc_ref, pneg_ref, bad_ref, ot_ref,
    x1_ref, st_ref, h2_ref, stage_ref,
):
    def copy(src, dst, sem):
        return pltpu.make_async_copy(src, dst, sem)

    cp_q = copy(wq_hbm, wq_ref, sems.at[0])
    cp_c = copy(c_hbm, c_ref.at[0], sems.at[1])
    cp_k = copy(wkt_hbm, wkv_ref.at[0], sems.at[2])
    cp_v = copy(wvt_hbm, wkv_ref.at[1], sems.at[3])
    cp_m0 = copy(wmod_hbm.at[:, pl.ds(0, MOD0)], wmod_ref.at[:, pl.ds(0, MOD0)], sems.at[4])
    cp_m1 = copy(wmod_hbm.at[:, pl.ds(MOD0, MOD1 - MOD0)], wmod_ref.at[:, pl.ds(MOD0, MOD1 - MOD0)],
                 sems.at[1])
    cp_x = [copy(xt_hbm.at[0, :, pl.ds(i * TM, TM)], xt_ref.at[i], sems.at[(0, 2, 3, 4, 0, 1, 5, 6)[i]])
            for i in range(NM)]
    cp_o = copy(wo_hbm, wo_ref, sems.at[0])
    cp_m2 = copy(wmod_hbm.at[:, pl.ds(MOD1, 6 * D - MOD1)], wmod_ref.at[:, pl.ds(MOD1, 6 * D - MOD1)],
                 sems.at[1])
    cp_w = [copy(w_hbm.at[:, pl.ds(fh * FH, FH)], w_ref.at[fh], sems.at[3 * fh + k])
            for fh in range(NFH)
            for k, (w_hbm, w_ref) in enumerate(((wg_hbm, wg_ref), (wu_hbm, wu_ref), (wdt_hbm, wdt_ref)))]

    for cp in [cp_q, cp_c, cp_k, cp_v, cp_m0]:
        cp.start()

    for cidx in range(NCH - LAG, NCH):
        s_ref[cidx % RING] = jnp.zeros((KC, TQ), F32)
    for slot in range(1, 4):
        sb_ref[slot] = jnp.zeros((NC, TQ), F32)
    pneg_ref[...] = jnp.zeros((8, TQ), F32)
    pacc_ref[...] = jnp.ones((VR, TQ), F32)
    bad_ref[...] = jnp.zeros((8, TQ), F32)

    def stats1(e):
        x = xt_ref[e // 2, :, (e % 2) * 128:(e % 2 + 1) * 128].astype(F32)
        mean, rstd = _stats(x)
        st_ref[e, 0:1, :] = mean
        st_ref[e, 8:9, :] = rstd
        return rstd

    cp_k.wait()
    cp_v.wait()
    cp_c.wait()
    zpad = jnp.zeros((KW - DH, D), F32)
    kv_t = jnp.concatenate(
        [wkv_ref[0].astype(F32), zpad, wkv_ref[1].astype(F32), zpad], axis=0)
    _pack_store(wqkv_ref, 0, kv_t)
    sc = jnp.broadcast_to(_silu(c_ref[0].astype(F32)), (8, D))
    cp_q.wait()
    cp_x[0].start()
    cp_m1.start()
    _pack_store(wqkv_ref, NKV, wq_ref[...].astype(F32).T)

    def mod_cols(lo, hi):
        mod = _dot(sc, wmod_ref[:, lo:hi])
        col = lo + jax.lax.broadcasted_iota(jnp.int32, (8, hi - lo), 1)
        scale = jnp.logical_or(jnp.logical_and(col >= D, col < 2 * D),
                               jnp.logical_and(col >= 4 * D, col < 5 * D))
        mod = jnp.where(scale, 1.0 + mod, mod)
        mod = mod * jnp.where(col >= 5 * D, 2.0, jnp.where(col >= 3 * D, 0.5, 1.0))
        mod_ref[lo:hi, :] = jnp.broadcast_to(mod[0:1, :], (128, hi - lo)).T

    cp_m0.wait()
    cp_x[1].start()
    mod_cols(0, MOD0)
    cp_x[0].wait()
    cp_x[2].start()
    cp_x[3].start()
    stats1(0)
    stats1(1)
    cp_m1.wait()
    for cp in cp_x[4:]:
        cp.start()
    mod_cols(MOD0, MOD1)

    def ln1(e, z=None):
        x = xt_ref[e // 2, :, (e % 2) * 128:(e % 2 + 1) * 128].astype(F32)
        mean = st_ref[e, 0:1, :] if z is None else st_ref[e, 0:1, :] + z
        h = ((x - mean) * (st_ref[e, 8:9, :] * mod_ref[D:2 * D, :])
             + mod_ref[0:D, :])
        h1_ref[e] = pltpu.bitcast(h.astype(BF16), jnp.int32)

    def proj_main(e):
        return _dot(_pack_load(wqkv_ref, 0, NQKV, 0, 512), pltpu.bitcast(h1_ref[e, 0:256, :], BF16))

    def proj_tail(qb):
        return _dot(_pack_load(wqkv_ref, 0, NQKV, 512, D),
                    _pack_load(h1_ref, 512, D, qb * TQ, (qb + 1) * TQ))

    def proj_out(e, qkv):
        tok = slice(e * KC, (e + 1) * KC)
        row = jax.lax.broadcasted_iota(jnp.int32, (VR, 128), 0)
        vt_ref[:, tok] = jnp.where(row == DH, 1.0, qkv[KW:NKV, :])
        kt = jnp.concatenate(
            [qkv[0:KW, :] * QK_SCALE, jnp.zeros((128 - KW, 128), F32)], axis=0)
        k = kt.T
        lane = jax.lax.broadcasted_iota(jnp.int32, (128, 128), 1)
        packed = [(MSZ[e] + 16 * n, 16 * g + (0 if kind == "v" else NV))
                  for n, (kind, g) in enumerate(TILES[e])]
        for r in range(4):
            kr = k if r == 0 else pltpu.roll(k, 2 * r, 1)
            kr = jnp.where(lane == ONE[r], 1.0, kr).astype(BF16)
            ks_ref[r, e * (KC // 2):(e + 1) * (KC // 2), :] = pltpu.bitcast(kr, jnp.int32)
            for src, dst in packed:
                if dst < NV or r == 0:
                    ksp_ref[r, dst:dst + 16, :] = kr[src:src + 16, :]
        for src, dst in packed:
            k0_ref[dst:dst + 16, :] = k[src:src + 16, :]
        for g in range(H // 4):
            lo = (g % 2) * TM + (e % 2) * 128
            qt_ref[(e // 2) * (SPB // 4) + g // 2, :, lo:lo + 128] = (
                qkv[NKV + g * 4 * DH:NKV + (g + 1) * 4 * DH, :])

    def q_window(t4, r, lanes=slice(None)):
        return qt_ref[t4, 16 * r:16 * r + KW, lanes]

    wrow = jax.lax.broadcasted_iota(jnp.int32, (KW, TQ), 0)

    def q_cols(t4, r, j):
        qw = q_window(t4, r, slice(j * 128, (j + 1) * 128))
        return jnp.stack(
            [jnp.broadcast_to(qw[2 * r + d:2 * r + d + 1, :], (8, 128)) for d in range(DH)])

    def vpu_scores(t4base, l4base, pieces, segs, zero, first_write):
        cur = None
        for (hh, j, kb), pin in zip(pieces, _pins(segs, len(pieces))):
            head = 4 * l4base + hh
            lanes = slice(j * 128, (j + 1) * 128)
            if cur != (hh, j):
                cur = (hh, j)
                qd = q_cols(t4base + hh // 4, hh % 4, j)
            sv = jnp.sum(kb_ref[:, kb * 8:(kb + 1) * 8, :] * qd, axis=0)
            if first_write:
                mask = None
                sv = sv + _tie(pin, zero)
            else:
                mask = _always(pin, zero)
            pltpu.store(sv_ref.at[head, kb * 8:(kb + 1) * 8, lanes], sv, mask=mask)
            if kb < NMX:
                m = sv if kb == 0 else jnp.maximum(m, sv)
            if kb == NMX - 1:
                pltpu.store(mv_ref.at[head, :, lanes], m, mask=mask)

    segs0 = []

    def sv_mxu(h):
        s = _dot(ksp_ref[h % 4, 0:NV, 0:KW],
                 jnp.where(wrow == ONE[h % 4], 0.0, q_window(h // 4, h % 4)))
        sv_ref[h] = s
        mv_ref[h] = _rowmax8(s[0:8 * NMX, :])
        segs0.append((s, 1.0))

    zero_a = (c_ref[0, :, 0:128].astype(F32) > 3e38).astype(jnp.int32) >> 1
    ln1(0)
    a = [proj_main(0)]
    ln1(1)
    cp_x[1].wait()
    a.append(proj_main(1))
    stats1(2)
    stats1(3)
    ln1(2)
    ln1(3, _tie(a[1][64:65, :], zero_a))
    tail = proj_tail(0)
    for e in range(2):
        proj_out(e, a[e] + tail[:, e * 128:(e + 1) * 128])
    cp_x[2].wait()
    cp_x[3].wait()
    for e in range(2, NCH):
        if e == 4:
            for cp in cp_x[4:]:
                cp.wait()
            cp_o.start()
            cp_m2.start()
        if e % 4 == 0:
            for n in range(e, e + 4):
                ln1(n)
            tail = proj_tail(e // 4)
        qkv = proj_main(e) + tail[:, (e % 4) * 128:(e % 4 + 1) * 128]
        nxt = {2: (4, 5), 3: (6, 7)}.get(e, (e + 4,) if e + 4 < NCH else ())
        for n, row in zip(nxt, (600, 320)):
            z = _tie(stats1(n), zero_a)
            qkv = jnp.concatenate([qkv[0:row, :], qkv[row:row + 8, :] + z, qkv[row + 8:, :]], axis=0)
        proj_out(e, qkv)
    cp_o.wait()
    cp_m2.wait()
    for cp in cp_w:
        cp.start()
    for d in range(DH):
        kb_ref[d] = jnp.broadcast_to(k0_ref[:, d:d + 1], (NV + NC, 128))
    for h in range(V0V, V0V + 4):
        sv_mxu(h)
    mod_cols(MOD1, 6 * D)
    _pack_store(wot_ref, 0, wo_ref[...].astype(F32).T)
    for h in range(V0V + 4, SPB):
        sv_mxu(h)
    sb_ref[0] = _dot(ksp_ref[0, NV:NV + NC, 0:KW], jnp.where(wrow == ONE[0], 0.0, q_window(0, 0)))
    vpu_scores(0, 0, [(hh, j, kb) for hh in range(V0V) for j in range(NTL) for kb in range(NV // 8)],
               segs0[V0S:], jnp.broadcast_to(zero_a, (8, 128)), True)

    def pv_tile(hs, cidx):
        parts = [s_ref[cidx % RING, 0:MSZ[cidx], :]]
        neg16 = jnp.concatenate([hs["neg"], hs["neg"]], axis=0)
        for kind, g in TILES[cidx]:
            rows = slice(g * 16, (g + 1) * 16)
            raw = sv_ref[hs["head"], rows, :] if kind == "v" else sb_ref[hs["u"] % 4, rows, :]
            parts.append(raw + neg16)
        p = jnp.exp2(jnp.concatenate(parts, axis=0)).astype(BF16)
        o = _dot(vt_ref[:, cidx * KC:(cidx + 1) * KC], p)
        hs["acc"] = o if hs["acc"] is None else hs["acc"] + o
        return o

    def store_o(g4, r, acc):
        ot_ref[g4, r * DH:(r + 1) * DH, :] = _normalize(acc)

    def flag(acc, bad):
        l = acc[16:24, :]
        ok = jnp.logical_and(l >= L_LO, l <= L_HI)
        row8 = jax.lax.broadcasted_iota(jnp.int32, (8, TQ), 0)
        return jnp.where(jnp.logical_or(ok, row8 != DH - 16), bad, 1.0)

    def attn_block(it):
        zero = jax.lax.shift_right_logical(it, 16)
        t4 = it * (HPI // 4)
        h0 = (it % IPB) * HPI
        bad = bad_ref[...]
        hs = {"acc": pacc_ref[...], "u": -1, "head": None, "neg": pneg_ref[...]}
        pend = [(hs, cidx) for cidx in range(NCH - LAG, NCH)]
        for u in range(HPI):
            r = u % 4
            mx = jnp.max(mv_ref[h0 + u], axis=0, keepdims=True)
            neg = jnp.broadcast_to(-mx, (8, TQ))
            neg = pltpu.bitcast(pltpu.bitcast(neg, jnp.int32) & jnp.int32(-65536), F32)
            q = jnp.where(wrow == ONE[r], jnp.concatenate([neg] * (KW // 8), axis=0),
                          q_window(t4 + u // 4, r))
            hs = {"acc": None, "u": u, "head": h0 + u, "neg": neg}
            rn = (u + 1) % 4
            tn4 = t4 + (u + 1) // 4
            if u == HPI - 1:
                tn4 = jnp.minimum(tn4, NT // 4 - 1)
            segs = []
            for cidx in range(NCH):
                kk = ks_ref[r, cidx * (KC // 2):cidx * (KC // 2) + MSZ[cidx] // 2, :]
                s = _dot(pltpu.bitcast(kk, BF16)[:, 0:KW], q)
                s_ref[cidx % RING, 0:MSZ[cidx], :] = s
                segs.append((s, MSZ[cidx] * (WB if cidx in (LAG - 1, LAG) else 1.0)))
                pend.append((hs, cidx))
                hp, cp = pend.pop(0)
                segs.append((pv_tile(hp, cp), WP * VR))
                if cp == NCH - 1:
                    g4 = t4 + hp["u"] // 4
                    if hp["u"] < 0:
                        g4 = jnp.maximum(g4, 0)
                    store_o(g4, hp["u"] % 4, hp["acc"])
                    bad = flag(hp["acc"], bad)
            for (j, kb), pin in zip(PIECES, _pins(segs, len(PIECES), 0.7, 0)):
                if kb == 0:
                    qd = q_cols(tn4, rn, j)
                sv = jnp.sum(kb_ref[:, NV + kb * 8:NV + (kb + 1) * 8, :] * qd, axis=0)
                pltpu.store(sb_ref.at[rn, kb * 8:(kb + 1) * 8, j * 128:(j + 1) * 128], sv,
                            mask=_always(pin, zero))
        pacc_ref[...] = hs["acc"]
        pneg_ref[...] = hs["neg"]
        bad_ref[...] = bad

    def attn_exact(mb):
        def head(h, carry):
            r = h % 4
            t4 = mb * (SPB // 4) + h // 4
            one = jnp.where(r == 3, ONE[3], ONE[0])
            q = jnp.where(wrow == one, 0.0, qt_ref[t4, pl.ds(pl.multiple_of(16 * r, 8), KW), :])

            def scores(cidx):
                kk = ks_ref[r, pl.ds(pl.multiple_of(cidx * (KC // 2), KC // 2), KC // 2), :]
                return _dot(pltpu.bitcast(kk, BF16)[:, 0:KW], q)

            m = jax.lax.fori_loop(
                0, NCH, lambda cidx, m: jnp.maximum(m, _rowmax8(scores(cidx))),
                jnp.full((8, TQ), -jnp.inf, F32))
            m = jnp.max(m, axis=0, keepdims=True)

            def pv(cidx, acc):
                p = jnp.exp2(scores(cidx) - m).astype(BF16)
                return acc + _dot(vt_ref[:, pl.ds(pl.multiple_of(cidx * KC, KC), KC)], p)

            acc = jax.lax.fori_loop(0, NCH, pv, jnp.zeros((VR, TQ), F32))
            for rr in range(4):
                @pl.when(r == rr)
                def _():
                    store_o(t4, rr, acc)
            return carry

        jax.lax.fori_loop(0, SPB, head, 0)

    def finish_block(mb):
        g0 = mb * (SPB // 4)
        zero = jax.lax.shift_right_logical(mb, 16)
        tn = jnp.minimum(mb + 1, NM - 1) * (SPB // 4)

        def o_rows(lo, hi):
            o = [ot_ref[g0 + g // 2, :, (g % 2) * TM:(g % 2 + 1) * TM]
                 for g in range(lo // (4 * DH), -(-hi // (4 * DH)))]
            off = lo // (4 * DH) * (4 * DH)
            return jnp.concatenate(o, axis=0)[lo - off:hi - off, :]

        def after(x, dep):
            z = jnp.concatenate([_tie(dep, zero)] * (x.shape[1] // 128), axis=1)
            return jnp.concatenate([x[0:-8, :], x[-8:, :] + z], axis=0)

        def resid(e, attn):
            x = xt_ref[mb, :, e * 128:(e + 1) * 128].astype(F32)
            x1 = x + mod_ref[2 * D:3 * D, :] * attn
            x1_ref[e] = x1
            return _stats(x1)

        def ln2(e, mean, rstd):
            x1 = x1_ref[e + zero]
            h2 = (x1 - mean) * (rstd * mod_ref[4 * D:5 * D, :]) + mod_ref[3 * D:4 * D, :]
            _pack_store(h2_ref, e * 128, h2.T)

        def project_rest(a, vpu=False):
            o = after(o_rows(512, D), a[256:264, 0:128])
            t = jnp.concatenate(
                [_dot(_pack_load(wot_ref, lo, lo + D // 2, 512, D), o) for lo in (0, D // 2)], axis=0)
            b = _dot(_pack_load(wot_ref, 0, D, 256, 512), after(o_rows(256, 512), t[32:40, 0:128]))
            attn = (a + t) + b
            if vpu:
                mine = [(hh + o, j, kb) for o in (0, SPB // NFH) for hh, j, kb in VPIECES[-FV:]]
                vpu_scores(tn, 0, mine,
                           [(a, float(D)), (t[0:D // 2, :], D / 2), (b, 0.3 * D)], zero, False)
            st = [resid(e, attn[:, e * 128:(e + 1) * 128]) for e in range(TM // 128)]
            for e in range(TM // 128):
                ln2(e, *st[e])

        def fill(steps):
            for h in steps:
                q = jnp.where(wrow == ONE[h % 4], 0.0, q_window(tn + h // 4, h % 4))
                sv_ref[h, NV - NVF:NV, :] = _dot(ksp_ref[h % 4, NV - NVF:NV, 0:KW], q)

        fill(range(NF0))
        hs = {"acc": pacc_ref[...], "u": -1, "head": None, "neg": pneg_ref[...]}
        for cidx in range(NCH - LAG, NCH):
            pv_tile(hs, cidx)
        a = _dot(_pack_load(wot_ref, 0, D, 0, 256), o_rows(0, 256))
        store_o(g0 + SPB // 4 - 1, 3, hs["acc"])
        bad = jnp.max(flag(hs["acc"], bad_ref[...]))
        bad_ref[...] = jnp.zeros((8, TQ), F32)
        project_rest(a, True)
        fill(range(NF0, SPB))

        @pl.when(bad > 0.0)
        def _():
            attn_exact(mb)
            project_rest(_dot(_pack_load(wot_ref, 0, D, 0, 256), o_rows(0, 256)))

    def out_copy(mb):
        return copy(stage_ref.at[mb], out_hbm.at[0, :, pl.ds(_aligned(mb * TM, TM), TM)],
                    sems.at[6])

    def ffn(i, carry):
        mb = i // NFH
        fh = i % NFH
        hm, ht = _pack_load(h2_ref, 0, TM, 0, 512), _pack_load(h2_ref, 0, TM, 512, D)
        segs = []
        acc = None
        ready = None
        pend = []

        def down(cols, a):
            if a.shape[1] == FU:
                y = _dot_nt(wdt_ref[fh, :, cols], a.astype(BF16))
                segs.append((y, float(D)))
                return y
            ys = [_dot_nt(wdt_ref[fh, :, cols], a[n * 128:(n + 1) * 128, :].astype(BF16))
                  for n in range(2)]
            segs.extend((y, float(D)) for y in ys)
            return jnp.concatenate(ys, axis=1)

        nu = FH // FU
        for un in range(nu):
            c0 = un * FU
            wt = jnp.concatenate(
                [wg_ref[fh, 512:D, c0:c0 + FU], wu_ref[fh, 512:D, c0:c0 + FU]], axis=1)
            t = _dot(ht, wt)
            segs.append((t, WT * TM))
            parts = []
            for n in range(2):
                cols = slice(c0 + n * 128, c0 + (n + 1) * 128)
                g = _dot(hm, wg_ref[fh, 0:512, cols])
                u = _dot(hm, wu_ref[fh, 0:512, cols])
                segs.extend([(g, float(TM)), (u, float(TM))])
                g = g + t[:, n * 128:(n + 1) * 128]
                u = u + t[:, FU + n * 128:FU + (n + 1) * 128]
                parts.append((g + g * jnp.tanh(g)) * u)
                if ready is not None and n == (1 if un == nu - 1 else 0):
                    y = down(*ready)
                    acc = y if acc is None else acc + y
                    ready = None
            pend.extend(parts)
            if len(pend) == 4 or un == nu - 1:
                a = jnp.concatenate(pend, axis=1)
                ready = (slice(c0 + FU - a.shape[1], c0 + FU), a)
                pend = []
        acc = acc + down(*ready)
        l4base = fh * (SPB // 4 // NFH)
        vpu_scores(jnp.minimum(mb + 1, NM - 1) * (SPB // 4) + l4base, l4base,
                   VPIECES[:-FV],
                   segs, jax.lax.shift_right_logical(i, 16), False)
        gb = mod_ref[5 * D:6 * D, :]
        for e in range(TM // 128):
            x2 = x1_ref[e] + gb * acc[:, e * 128:(e + 1) * 128]
            x1_ref[e] = x2
            stage_ref[mb, :, e * 128:(e + 1) * 128] = x2.astype(BF16)

        @pl.when(fh == NFH - 1)
        def _():
            out_copy(mb).start()

        return carry

    def main_loop(it, carry):
        attn_block(it)

        @pl.when(it % IPB == IPB - 1)
        def _():
            mb = it // IPB
            finish_block(mb)

            @pl.when(mb == 0)
            def _():
                for cp in cp_w:
                    cp.wait()

            jax.lax.fori_loop(mb * NFH, (mb + 1) * NFH, ffn, 0)

        return carry

    jax.lax.fori_loop(0, NT // HPI, main_loop, 0)
    for mb in range(NM):
        out_copy(mb).wait()


@jax.jit
def pallas_adaLN_cond__grouped_kv_mqa__swiglu_ffn__prompt_kernel(
    A_x: jax.Array,
    A_wq: jax.Array,
    A_wk: jax.Array,
    A_wv: jax.Array,
    A_wo: jax.Array,
    B_x: jax.Array,
    B_w_gate: jax.Array,
    B_w_up: jax.Array,
    B_w_down: jax.Array,
    c: jax.Array,
    w_mod: jax.Array,
):
    del B_x
    hbm = pl.BlockSpec(memory_space=pltpu.HBM)
    out_t = pl.pallas_call(
        _kernel,
        out_shape=jax.ShapeDtypeStruct((1, D, S), A_x.dtype),
        in_specs=[hbm] * 10,
        out_specs=hbm,
        scratch_shapes=[
            pltpu.VMEM((NM, D, TM), BF16),
            pltpu.VMEM((D, D), BF16),
            pltpu.VMEM((8, DH, D), BF16),
            pltpu.VMEM((D, D), BF16),
            pltpu.VMEM((NFH, D, FH), BF16),
            pltpu.VMEM((NFH, D, FH), BF16),
            pltpu.VMEM((NFH, D, FH), BF16),
            pltpu.VMEM((32, 1, D), BF16),
            pltpu.VMEM((D, 6 * D), BF16),
            pltpu.SemaphoreType.DMA((7,)),
            pltpu.VMEM((6 * D, 128), F32),
            pltpu.VMEM((5, 320, 128), jnp.int32),
            pltpu.VMEM((5, D // 2, 128), jnp.int32),
            pltpu.VMEM((NCH, D // 2, 128), jnp.int32),
            pltpu.VMEM((4, S // 2, 128), jnp.int32),
            pltpu.VMEM((4, NV + NC, 128), BF16),
            pltpu.VMEM((NV + NC, 128), F32),
            pltpu.VMEM((DH, NV + NC, 128), F32),
            pltpu.VMEM((VR, S), F32),
            pltpu.VMEM((NT // 4, 4 * DH, TQ), F32),
            pltpu.VMEM((RING, KC, TQ), F32),
            pltpu.VMEM((SPB, NV, TQ), F32),
            pltpu.VMEM((SPB, 8, TQ), F32),
            pltpu.VMEM((4, NC, TQ), F32),
            pltpu.VMEM((VR, TQ), F32),
            pltpu.VMEM((8, TQ), F32),
            pltpu.VMEM((8, TQ), F32),
            pltpu.VMEM((NT // 4, 4 * DH, TQ), F32),
            pltpu.VMEM((TM // 128, D, 128), F32),
            pltpu.VMEM((16, 16, 128), F32),
            pltpu.VMEM((5, TM // 2, 128), jnp.int32),
            pltpu.VMEM((NM, D, TM), BF16),
        ],
        compiler_params=pltpu.CompilerParams(
            vmem_limit_bytes=100 * 1024 * 1024, internal_scratch_in_bytes=65536),
    )(
        jnp.transpose(A_x, (0, 2, 1)), A_wq, A_wk.T, A_wv.T, A_wo,
        B_w_gate, B_w_up, B_w_down.T, c, w_mod,
    )
    return jnp.transpose(out_t, (0, 2, 1))
```
